```python
import jax
import jax.numpy as jnp

def _softmax(x, axis=-1):
    return jax.nn.softmax(x, axis=axis)
def _gelu(x):
    return jax.nn.gelu(x, approximate=True)
def _silu(x):
    return jax.nn.silu(x)
def _sigmoid(x):
    return jax.nn.sigmoid(x)
def _layernorm(x, axis=-1, eps=1e-5):
    m = jnp.mean(x, axis=axis, keepdims=True)
    v = jnp.var(x, axis=axis, keepdims=True)
    return (x - m) / jnp.sqrt(v + eps)
def _scatter_add(tgt, idx, src, axis=0):
    return tgt.at[idx].add(src)
def _segment_sum(src, seg, n):
    return jax.ops.segment_sum(src, seg, n)
class _Rng:
    def __init__(self, key):
        self._k = key
    def _next(self):
        self._k, sub = jax.random.split(self._k)
        return sub
    def normal(self, shape):
        return jax.random.normal(self._next(), shape, dtype=jnp.bfloat16)
    def randint(self, lo, hi, shape):
        return jax.random.randint(self._next(), shape, lo, hi, dtype=jnp.int32)
    def uniform(self, shape, lo=0.0, hi=1.0):
        return jax.random.uniform(self._next(), shape, jnp.bfloat16, lo, hi)
    def permutation(self, n):
        return jax.random.permutation(self._next(), n)


kernel_name = 'recurrent_scan__gqa_block_cached__moe_arch_mod__prompt'

def setup_inputs():
    _rng = _Rng(jax.random.key(int.from_bytes(__import__("os").urandom(4), "little")))
    _w = (lambda a: (lambda t: t.astype(jnp.bfloat16) if jnp.issubdtype(t.dtype, jnp.floating) else t)(jnp.asarray(a)))
    def _A_setup():
        B, Sq, D = 1, 2048, 576
        Hq, Hkv, Sk, Dh = 32, 16, 2048, 128
        assert Hq % Hkv == 0, (Hq, Hkv)
        return {
            "x": _w((lambda *s: _rng.normal(s) * 0.05)(B, Sq, D)),
            "k_cache": _w((lambda *s: _rng.normal(s) * 0.05)(B, Hkv, Sk, Dh)),
            "v_cache": _w((lambda *s: _rng.normal(s) * 0.05)(B, Hkv, Sk, Dh)),
            "wq": _w((lambda *s: _rng.normal(s) * 0.05)(D, Hq * Dh) * (D ** -0.5)),
            "wo": _w((lambda *s: _rng.normal(s) * 0.05)(Hq * Dh, D) * ((Hq * Dh) ** -0.5)),
        }
    _A_in = _A_setup()

    def _B_setup():
        B, S, D, F, C = 1, 2048, 576, 4608, 8
        return {
            "x": _w((lambda *s: _rng.normal(s) * 0.05)(B, S, D)),
            "w_r": _w((lambda *s: _rng.normal(s) * 0.05)(D)),
            "w_gate": _w((lambda *s: _rng.normal(s) * 0.05)(D, F)),
            "w_up": _w((lambda *s: _rng.normal(s) * 0.05)(D, F)),
            "w_down": _w((lambda *s: _rng.normal(s) * 0.05)(F, D)),
        }
    _B_in = _B_setup()

    return {
        "A_x": _A_in["x"],
        "A_k_cache": _A_in["k_cache"],
        "A_v_cache": _A_in["v_cache"],
        "A_wq": _A_in["wq"],
        "A_wo": _A_in["wo"],
        "B_x": _B_in["x"],
        "B_w_r": _B_in["w_r"],
        "B_w_gate": _B_in["w_gate"],
        "B_w_up": _B_in["w_up"],
        "B_w_down": _B_in["w_down"],
    }

def reference(A_x, A_k_cache, A_v_cache, A_wq, A_wo, B_x, B_w_r, B_w_gate, B_w_up, B_w_down):
    def _A_ref(x, k_cache, v_cache, wq, wo):
        B, Sq, D = x.shape
        Hq, Dh = 32, 128
        Hkv = k_cache.shape[1]
        rep = Hq // Hkv
        q = (lambda x, *d: x.transpose(*d))((x @ wq).reshape(B, Sq, Hq, Dh), 0, 2, 1, 3)
        k = jnp.repeat(k_cache, rep, axis=1)
        v = jnp.repeat(v_cache, rep, axis=1)
        scores = jnp.einsum("bhqd,bhkd->bhqk", q, k) * (Dh ** -0.5)
        p = _softmax(scores, axis=-1)
        o = jnp.einsum("bhqk,bhkd->bhqd", p, v)
        return (lambda x, *d: x.transpose(*d))(o, 0, 2, 1, 3).reshape(B, Sq, Hq * Dh) @ wo

    def _B_ref(x, w_r, w_gate, w_up, w_down):
        B, S, D = x.shape
        C = 8
        r = x @ w_r
        idx = jnp.argsort(-r, axis=-1)[:, :C]
        idx_e = jnp.repeat(idx.reshape(B, C, 1), D, axis=2)
        x_sel = jnp.take_along_axis(x, idx_e, axis=1)
        g = _silu(x_sel @ w_gate)
        u = x_sel @ w_up
        y = (g * u) @ w_down
        r_sel = _sigmoid(jnp.take_along_axis(r, idx, axis=1))
        y = y * r_sel.reshape(B, C, 1)
        b_off = (jnp.arange(B) * S).reshape(B, 1)
        flat_idx = (idx + b_off).reshape(B * C)
        zero = (x * 0.0).reshape(B * S, D)
        upd = _scatter_add(zero, flat_idx, y.reshape(B * C, D), axis=0)
        return x + upd.reshape(B, S, D)

    x = A_x
    xn = _layernorm(x, axis=-1)
    s = _A_ref(xn, A_k_cache, A_v_cache, A_wq, A_wo)
    g = _silu(_B_ref(xn, B_w_r, B_w_gate, B_w_up, B_w_down))
    return x + s * g
```

```python
import functools
import math

import jax
import jax.numpy as jnp
import jax.experimental.pallas as pl
import jax.experimental.pallas.tpu as pltpu

_BF16 = jnp.bfloat16
_F32 = jnp.float32

S = 2048
D = 576
HQ = 32
HKV = 16
DH = 128
REP = HQ // HKV
F = 4608
C = 8
CP = 16
EPS = 1e-5

TQ = 256
NCH = S // TQ
FC = 384
NF = F // FC
QSCALE = (DH ** -0.5) * math.log2(math.e)

_NT = (((1,), (1,)), ((), ()))


def _rb(x):
    return x.astype(_BF16).astype(_F32)


def _tree(a, op):
    tiles = [a[:, i * 128:(i + 1) * 128] for i in range(a.shape[1] // 128)]
    while len(tiles) > 1:
        tiles = [op(tiles[i], tiles[i + 1]) for i in range(0, len(tiles), 2)]
    return tiles[0]


def _kernel(xt_ref, k_ref, v_ref, wq_ref, wot_ref, wr_ref, wg_ref, wu_ref, wdt_ref,
            out_ref,
            xn_ref, xnt_ref, acc_ref, sel_ref, xsel_ref, rsel_ref, y_ref):
    g = pl.program_id(0)

    @pl.when(g == 0)
    def _prologue():
        for c in range(NCH):
            cols = pl.ds(c * TQ, TQ)
            x = xt_ref[:, cols].astype(_F32)
            mean = jnp.sum(x, axis=0, keepdims=True) * (1.0 / D)
            xc = x - mean
            var = jnp.sum(xc * xc, axis=0, keepdims=True) * (1.0 / D)
            num = _rb(x - _rb(mean))
            den = _rb(jnp.sqrt(_rb(_rb(var) + EPS)))
            xn = _rb(num / den)
            xnt_ref[:, cols] = xn.astype(_BF16)
            xn_ref[cols, :] = xn.T.astype(_BF16)
            acc_ref[:, cols] = jnp.zeros((D, TQ), _F32)
        wr = jnp.broadcast_to(wr_ref[...].reshape(1, D), (8, D))
        r = jnp.dot(wr, xnt_ref[...], preferred_element_type=_F32)
        r = _rb(r[0:1, :])
        pos = jax.lax.broadcasted_iota(jnp.int32, (1, S), 1)
        sels, rsel = [], []
        for c in range(C):
            m = jnp.max(r, axis=1, keepdims=True)
            idx = jnp.min(jnp.where(r == m, pos, S), axis=1, keepdims=True)
            hit = pos == idx
            sels.append(hit.astype(_F32))
            rsel.append(jnp.broadcast_to(m, (1, 128)))
            r = jnp.where(hit, -jnp.inf, r)
        sel = jnp.concatenate(sels + [jnp.zeros((CP - C, S), _F32)], axis=0)
        sel_ref[...] = sel.astype(_BF16)
        rsel_ref[...] = jnp.concatenate(rsel + [jnp.zeros((CP - C, 128), _F32)], axis=0)
        xsel_ref[...] = jax.lax.dot_general(
            sel.astype(_BF16), xnt_ref[...], _NT,
            preferred_element_type=_F32).astype(_BF16)
        y_ref[...] = jnp.zeros_like(y_ref)

    @pl.when(g < NF)
    def _moe():
        xs = xsel_ref[...]
        gate = jnp.dot(xs, wg_ref[...], preferred_element_type=_F32)
        up = jnp.dot(xs, wu_ref[...], preferred_element_type=_F32)
        h = (gate * jax.nn.sigmoid(gate)) * up
        y_ref[...] += jax.lax.dot_general(h.astype(_BF16), wdt_ref[...], _NT,
                                          preferred_element_type=_F32)

    k = k_ref[...]
    v = v_ref[...]

    def qproj(c):
        q = jnp.dot(xn_ref[pl.ds(c * TQ, TQ), :], wq_ref[...], preferred_element_type=_F32)
        return (q * QSCALE).astype(_BF16)

    def qk(q, h):
        return jax.lax.dot_general(q[:, h * DH:(h + 1) * DH], k, _NT, preferred_element_type=_F32)

    def pv(s):
        m = jnp.max(_tree(s, jnp.maximum), axis=-1, keepdims=True)
        p = jnp.exp2(s - m)
        tiles = [p[:, i * 128:(i + 1) * 128] for i in range(S // 128)]
        acc = None
        for g0 in range(0, len(tiles), 4):
            t = (tiles[g0] + tiles[g0 + 1]) + (tiles[g0 + 2] + tiles[g0 + 3])
            acc = t if acc is None else acc + t
            tiles[g0 + 3] = jnp.minimum(tiles[g0 + 3], acc)
        l = jnp.sum(acc, axis=-1, keepdims=True)
        pb = jnp.concatenate(tiles, axis=-1).astype(_BF16)
        o = jnp.dot(pb, v, preferred_element_type=_F32)
        r = pl.reciprocal(l, approx=True)
        r = r * (2.0 - l * r)
        return (o * r).astype(_BF16)

    def oproj(c, oa, ob):
        o2 = jnp.concatenate([oa, ob], axis=-1)
        acc_ref[:, pl.ds(c * TQ, TQ)] += jax.lax.dot_general(
            wot_ref[...], o2, _NT, preferred_element_type=_F32)

    qs = [qproj(c) for c in range(NCH)]
    outs = []
    for c in range(NCH):
        outs.append((pv(qk(qs[c], 0)), pv(qk(qs[c], 1))))
    for c in range(NCH):
        oproj(c, *outs[c])

    @pl.when(g == HKV - 1)
    def _epilogue():
        y = y_ref[...] * jax.nn.sigmoid(rsel_ref[:, 0:1])
        yt = jnp.concatenate([y, jnp.zeros((128 - CP, D), _F32)], axis=0).T
        yt = yt.astype(_BF16)
        for c in range(NCH):
            cols = pl.ds(c * TQ, TQ)
            selc = jnp.concatenate(
                [sel_ref[:, cols], jnp.zeros((128 - CP, TQ), _BF16)], axis=0)
            upd = jnp.dot(yt, selc, preferred_element_type=_F32)
            b = xnt_ref[:, cols].astype(_F32) + upd
            gate = b * jax.nn.sigmoid(b)
            out_ref[:, cols] = (xt_ref[:, cols].astype(_F32)
                                + acc_ref[:, cols] * gate).astype(out_ref.dtype)


@jax.jit
def pallas_recurrent_scan__gqa_block_cached__moe_arch_mod__prompt_kernel(
    A_x: jax.Array,
    A_k_cache: jax.Array,
    A_v_cache: jax.Array,
    A_wq: jax.Array,
    A_wo: jax.Array,
    B_x: jax.Array,
    B_w_r: jax.Array,
    B_w_gate: jax.Array,
    B_w_up: jax.Array,
    B_w_down: jax.Array,
):
    xt = A_x.reshape(S, D).T
    k = A_k_cache.reshape(HKV, S, DH)
    v = A_v_cache.reshape(HKV, S, DH)
    wot = A_wo.T
    wdt = B_w_down.T

    fidx = lambda g: jnp.minimum(g, NF - 1)
    in_specs = [
        pl.BlockSpec((D, S), lambda g: (0, 0)),
        pl.BlockSpec((None, S, DH), lambda g: (g, 0, 0)),
        pl.BlockSpec((None, S, DH), lambda g: (g, 0, 0)),
        pl.BlockSpec((D, REP * DH), lambda g: (0, g)),
        pl.BlockSpec((D, REP * DH), lambda g: (0, g)),
        pl.BlockSpec((D,), lambda g: (0,)),
        pl.BlockSpec((D, FC), lambda g: (0, fidx(g))),
        pl.BlockSpec((D, FC), lambda g: (0, fidx(g))),
        pl.BlockSpec((D, FC), lambda g: (0, fidx(g))),
    ]
    out_t = pl.pallas_call(
        _kernel,
        grid=(HKV,),
        in_specs=in_specs,
        out_specs=pl.BlockSpec((D, S), lambda g: (0, 0)),
        out_shape=jax.ShapeDtypeStruct((D, S), A_x.dtype),
        scratch_shapes=[
            pltpu.VMEM((S, D), _BF16),
            pltpu.VMEM((D, S), _BF16),
            pltpu.VMEM((D, S), _F32),
            pltpu.VMEM((CP, S), _BF16),
            pltpu.VMEM((CP, D), _BF16),
            pltpu.VMEM((CP, 128), _F32),
            pltpu.VMEM((CP, D), _F32),
        ],
        compiler_params=pltpu.CompilerParams(
            dimension_semantics=("arbitrary",),
            vmem_limit_bytes=126 * 1024 * 1024,
        ),
        name="fused_gqa_mod",
    )(xt, k, v, A_wq, wot, B_w_r, B_w_gate, B_w_up, wdt)
    return out_t.T.reshape(1, S, D)
```

```python
import math

import jax
import jax.numpy as jnp
import jax.experimental.pallas as pl
import jax.experimental.pallas.tpu as pltpu

_BF16 = jnp.bfloat16
_F32 = jnp.float32
_I32 = jnp.int32

S = 2048
D = 576
HQ = 32
HKV = 16
DH = 128
REP = HQ // HKV
GW = REP * DH
F = 4608
C = 8
CP = 16
EPS = 1e-5

TQ = 256
NCH = S // TQ
FC = 384
NF = F // FC
XDEPTH = 2
QSCALE = (DH ** -0.5) * math.log2(math.e)

_NT = (((1,), (1,)), ((), ()))


def _rb(x):
    return x.astype(_BF16).astype(_F32)


def _recip(x):
    r = pl.reciprocal(x, approx=True)
    return r * (2.0 - x * r)


def _tree(a, op):
    tiles = [a[:, i * 128:(i + 1) * 128] for i in range(a.shape[1] // 128)]
    while len(tiles) > 1:
        tiles = [op(tiles[i], tiles[i + 1]) for i in range(0, len(tiles), 2)]
    return tiles[0]


def _kernel(xt_hbm, k_hbm, v_hbm, wq_hbm, wot_hbm, wr_hbm, wg_hbm, wu_hbm, wdt_hbm,
            out_hbm,
            xt_ref, wr_ref, kbuf, vbuf, wqbuf, wobuf, wgbuf, wubuf, wdbuf, obuf,
            xn_ref, xnt_ref, acc_ref, sel_ref, xsel_ref, rsel_ref, y_ref,
            raw_ref, x_sem, o_sem, w_sem, a_sem, m_sem):
    g = pl.program_id(0)
    slot = g % 2

    def x_copy(c):
        cols = pl.ds(c * TQ, TQ)
        return pltpu.make_async_copy(xt_hbm.at[:, cols], xt_ref.at[:, cols], x_sem.at[c])

    def out_copy(c):
        cols = pl.ds(c * TQ, TQ)
        return pltpu.make_async_copy(obuf.at[:, cols], out_hbm.at[:, cols], o_sem.at[c])

    def wr_copy():
        return pltpu.make_async_copy(wr_hbm, wr_ref, w_sem.at[0])

    def attn_copies(h, s):
        cols = pl.ds(pl.multiple_of(h * GW, GW), GW)
        return [
            pltpu.make_async_copy(wq_hbm.at[:, cols], wqbuf.at[s], a_sem.at[s, 0]),
            pltpu.make_async_copy(k_hbm.at[h], kbuf.at[s], a_sem.at[s, 1]),
            pltpu.make_async_copy(v_hbm.at[h], vbuf.at[s], a_sem.at[s, 2]),
            pltpu.make_async_copy(wot_hbm.at[:, cols], wobuf.at[h % 3], a_sem.at[s, 3]),
        ]

    def moe_copies(j, s):
        cols = pl.ds(pl.multiple_of(j * FC, 128), FC)
        return [
            pltpu.make_async_copy(wg_hbm.at[:, cols], wgbuf.at[s], m_sem.at[s, 0]),
            pltpu.make_async_copy(wu_hbm.at[:, cols], wubuf.at[s], m_sem.at[s, 1]),
            pltpu.make_async_copy(wdt_hbm.at[:, cols], wdbuf.at[s], m_sem.at[s, 2]),
        ]

    @pl.when(g == 0)
    def _prologue():
        wr_copy().start()
        for c in range(XDEPTH):
            x_copy(c).start()
        wr_copy().wait()
        wr = jnp.broadcast_to(wr_ref[...].reshape(1, D), (8, D))
        rs = []
        for c in range(NCH):
            cols = pl.ds(c * TQ, TQ)
            x_copy(c).wait()
            if c + XDEPTH < NCH:
                x_copy(c + XDEPTH).start()
            if c == NCH - 3:
                for cp in attn_copies(0, 0):
                    cp.start()
            x = xt_ref[:, cols].astype(_F32)
            d = x - x[0:1, :]
            md = jnp.sum(d, axis=0, keepdims=True) * (1.0 / D)
            var = jnp.sum(d * d, axis=0, keepdims=True) * (1.0 / D) - md * md
            var = jnp.maximum(var, 0.0)
            mean = x[0:1, :] + md
            den = _rb(jnp.sqrt(_rb(_rb(var) + EPS)))
            xn32 = _rb(x - _rb(mean)) * _recip(den)
            xn = xn32.astype(_BF16)
            xnt_ref[:, cols] = xn
            xn_ref[cols, :] = xn32.T.astype(_BF16)
            rs.append(jnp.dot(wr, xn, preferred_element_type=_F32)[0:1, :])
        r = _rb(jnp.concatenate(rs, axis=1)) + 0.0
        pos = jax.lax.broadcasted_iota(_I32, (1, S), 1)
        bits = pltpu.bitcast(r, _I32)
        key = jnp.where(bits < 0, bits ^ 0x7FFF0000, bits) | (S - 1 - pos)
        row16 = jax.lax.broadcasted_iota(_I32, (16, D), 0)
        sels, rsel, xsel = [], [], []
        for c in range(C):
            m = jnp.max(key, axis=1, keepdims=True)
            hit = key == m
            sels.append(hit.astype(_F32))
            hi = jnp.broadcast_to(m, (1, 128)) & jnp.int32(-65536)
            rsel.append(pltpu.bitcast(jnp.where(hi < 0, hi ^ 0x7FFF0000, hi), _F32))
            key = jnp.where(hit, jnp.iinfo(jnp.int32).min, key)
            idx = (S - 1) - (m[0, 0] & (S - 1))
            blk = xn_ref[pl.ds(pl.multiple_of((idx // 16) * 16, 16), 16), :].astype(_F32)
            xsel.append(jnp.sum(jnp.where(row16 == idx % 16, blk, 0.0), axis=0, keepdims=True))
        sel_ref[...] = jnp.concatenate(
            sels + [jnp.zeros((CP - C, S), _F32)], axis=0).astype(_BF16)
        rsel_ref[...] = jnp.concatenate(rsel + [jnp.zeros((CP - C, 128), _F32)], axis=0)
        xsel_ref[...] = jnp.concatenate(
            xsel + [jnp.zeros((CP - C, D), _F32)], axis=0).astype(_BF16)
        y_ref[...] = jnp.zeros_like(y_ref)
        wobuf[2] = jnp.zeros((D, GW), _BF16)
        for h in range(REP):
            raw_ref[h, 0] = jnp.zeros((TQ, 128), _F32)
            raw_ref[h, 1] = jnp.ones((TQ, 128), _F32)

    @pl.when(g + 1 < HKV)
    def _prefetch_attn():
        for cp in attn_copies(g + 1, 1 - slot):
            cp.start()

    @pl.when(g < NF)
    def _prefetch_moe():
        for cp in moe_copies(g, 1 - slot):
            cp.start()

    @pl.when(jnp.logical_and(g >= 1, g <= NF))
    def _moe():
        for cp in moe_copies(g - 1, slot):
            cp.wait()
        xs = xsel_ref[...]
        gate = jnp.dot(xs, wgbuf[slot], preferred_element_type=_F32)
        up = jnp.dot(xs, wubuf[slot], preferred_element_type=_F32)
        h = (gate * jax.nn.sigmoid(gate)) * up
        y_ref[...] += jax.lax.dot_general(h.astype(_BF16), wdbuf[slot], _NT,
                                          preferred_element_type=_F32)

    for cp in attn_copies(g, slot):
        cp.wait()

    k = kbuf[slot]
    v = vbuf[slot]

    def qproj(c):
        q = jnp.dot(xn_ref[pl.ds(c * TQ, TQ), :], wqbuf[slot], preferred_element_type=_F32)
        return (q * QSCALE).astype(_BF16)

    def qk(q, h):
        return jax.lax.dot_general(q[:, h * DH:(h + 1) * DH], k, _NT, preferred_element_type=_F32)

    def normalize(o, part):
        l = jnp.sum(part, axis=-1, keepdims=True)
        return (o * _recip(l)).astype(_BF16)

    def pv(s):
        m = jnp.max(_tree(s, jnp.maximum), axis=-1, keepdims=True)
        p = jnp.exp2(s - m)
        tiles = [p[:, i * 128:(i + 1) * 128] for i in range(S // 128)]
        acc = None
        for g0 in range(0, len(tiles), 4):
            t = (tiles[g0] + tiles[g0 + 1]) + (tiles[g0 + 2] + tiles[g0 + 3])
            acc = t if acc is None else acc + t
            tiles[g0 + 3] = jnp.minimum(tiles[g0 + 3], acc)
        pb = jnp.concatenate(tiles, axis=-1).astype(_BF16)
        return jnp.dot(pb, v, preferred_element_type=_F32), acc

    def oproj(c, oa, ob, wo, first):
        o2 = jnp.concatenate([oa, ob], axis=-1)
        cols = pl.ds(c * TQ, TQ)
        prev = acc_ref[:, cols]
        if first:
            prev = jnp.where(g > 0, prev, 0.0)
        acc_ref[:, cols] = prev + jax.lax.dot_general(
            wo, o2, _NT, preferred_element_type=_F32)

    def deferred_oproj(wo, first):
        oa = normalize(raw_ref[0, 0], raw_ref[0, 1])
        ob = normalize(raw_ref[1, 0], raw_ref[1, 1])
        oproj(NCH - 1, oa, ob, wo, first)

    qs = [qproj(c) for c in range(NCH)]
    deferred_oproj(wobuf[(g + 2) % 3], True)
    outs = []
    for c in range(NCH):
        sa = qk(qs[c], 0)
        sb = qk(qs[c], 1)
        ra, rb_ = pv(sa), pv(sb)
        if c < NCH - 1:
            outs.append((normalize(*ra), normalize(*rb_)))
        else:
            for h, r in enumerate((ra, rb_)):
                raw_ref[h, 0] = r[0]
                raw_ref[h, 1] = r[1]
    wo_cur = wobuf[g % 3]
    for c in range(NCH - 1):
        oproj(c, *outs[c], wo_cur, True)

    @pl.when(g == HKV - 1)
    def _epilogue():
        y = y_ref[...] * jax.nn.sigmoid(rsel_ref[:, 0:1])
        yt = jnp.concatenate([y, jnp.zeros((128 - CP, D), _F32)], axis=0).T
        yt = yt.astype(_BF16)
        for c in range(NCH):
            cols = pl.ds(c * TQ, TQ)
            if c == NCH - 1:
                deferred_oproj(wobuf[(HKV - 1) % 3], False)
            selc = jnp.concatenate(
                [sel_ref[:, cols], jnp.zeros((128 - CP, TQ), _BF16)], axis=0)
            upd = jnp.dot(yt, selc, preferred_element_type=_F32)
            hb = 0.5 * (xnt_ref[:, cols].astype(_F32) + upd)
            gate = hb + hb * jnp.tanh(hb)
            obuf[:, cols] = (xt_ref[:, cols].astype(_F32)
                             + acc_ref[:, cols] * gate).astype(_BF16)
            out_copy(c).start()
        for c in range(NCH):
            out_copy(c).wait()


@jax.jit
def pallas_recurrent_scan__gqa_block_cached__moe_arch_mod__prompt_kernel(
    A_x: jax.Array,
    A_k_cache: jax.Array,
    A_v_cache: jax.Array,
    A_wq: jax.Array,
    A_wo: jax.Array,
    B_x: jax.Array,
    B_w_r: jax.Array,
    B_w_gate: jax.Array,
    B_w_up: jax.Array,
    B_w_down: jax.Array,
):
    xt = A_x.reshape(S, D).T
    k = A_k_cache.reshape(HKV, S, DH)
    v = A_v_cache.reshape(HKV, S, DH)
    wot = A_wo.T
    wdt = B_w_down.T

    out_t = pl.pallas_call(
        _kernel,
        grid=(HKV,),
        in_specs=[pl.BlockSpec(memory_space=pl.ANY)] * 9,
        out_specs=pl.BlockSpec(memory_space=pl.ANY),
        out_shape=jax.ShapeDtypeStruct((D, S), A_x.dtype),
        scratch_shapes=[
            pltpu.VMEM((D, S), _BF16),
            pltpu.VMEM((D,), _BF16),
            pltpu.VMEM((2, S, DH), _BF16),
            pltpu.VMEM((2, S, DH), _BF16),
            pltpu.VMEM((2, D, GW), _BF16),
            pltpu.VMEM((3, D, GW), _BF16),
            pltpu.VMEM((2, D, FC), _BF16),
            pltpu.VMEM((2, D, FC), _BF16),
            pltpu.VMEM((2, D, FC), _BF16),
            pltpu.VMEM((D, S), _BF16),
            pltpu.VMEM((S, D), _BF16),
            pltpu.VMEM((D, S), _BF16),
            pltpu.VMEM((D, S), _F32),
            pltpu.VMEM((CP, S), _BF16),
            pltpu.VMEM((CP, D), _BF16),
            pltpu.VMEM((CP, 128), _F32),
            pltpu.VMEM((CP, D), _F32),
            pltpu.VMEM((REP, 2, TQ, 128), _F32),
            pltpu.SemaphoreType.DMA((NCH,)),
            pltpu.SemaphoreType.DMA((NCH,)),
            pltpu.SemaphoreType.DMA((1,)),
            pltpu.SemaphoreType.DMA((2, 4)),
            pltpu.SemaphoreType.DMA((2, 3)),
        ],
        compiler_params=pltpu.CompilerParams(
            dimension_semantics=("arbitrary",),
            vmem_limit_bytes=126 * 1024 * 1024,
        ),
        name="fused_gqa_mod",
    )(xt, k, v, A_wq, wot, B_w_r, B_w_gate, B_w_up, wdt)
    return out_t.T.reshape(1, S, D)
```

```python
import math

import jax
import jax.numpy as jnp
import jax.experimental.pallas as pl
import jax.experimental.pallas.tpu as pltpu

_BF16 = jnp.bfloat16
_F32 = jnp.float32
_I32 = jnp.int32

S = 2048
D = 576
HQ = 32
HKV = 16
DH = 128
REP = HQ // HKV
GW = REP * DH
F = 4608
C = 8
CP = 16
EPS = 1e-5

TQ = 256
NCH = S // TQ
FC = 384
NF = F // FC
XDEPTH = 2
QSCALE = (DH ** -0.5) * math.log2(math.e)

_NT = (((1,), (1,)), ((), ()))


def _rb(x):
    return x.astype(_BF16).astype(_F32)


def _recip(x):
    r = pl.reciprocal(x, approx=True)
    return r * (2.0 - x * r)


def _tree(a, op):
    tiles = [a[:, i * 128:(i + 1) * 128] for i in range(a.shape[1] // 128)]
    while len(tiles) > 1:
        tiles = [op(tiles[i], tiles[i + 1]) for i in range(0, len(tiles), 2)]
    return tiles[0]


def _kernel(xt_hbm, k_hbm, v_hbm, wq_hbm, wot_hbm, wr_hbm, wg_hbm, wu_hbm, wdt_hbm,
            out_hbm,
            xt_ref, wr_ref, kbuf, vbuf, wqbuf, wobuf, wgbuf, wubuf, wdbuf, obuf,
            xn_ref, xnt_ref, acc_ref, sel_ref, xsel_ref, rsel_ref, y_ref,
            raw_ref, x_sem, o_sem, w_sem, a_sem, m_sem):
    g = pl.program_id(0)
    slot = g % 2

    def x_copy(c):
        cols = pl.ds(c * TQ, TQ)
        return pltpu.make_async_copy(xt_hbm.at[:, cols], xt_ref.at[:, cols], x_sem.at[c])

    def out_copy(c):
        cols = pl.ds(c * TQ, TQ)
        return pltpu.make_async_copy(obuf.at[:, cols], out_hbm.at[:, cols], o_sem.at[c])

    def wr_copy():
        return pltpu.make_async_copy(wr_hbm, wr_ref, w_sem.at[0])

    def attn_copies(h, s):
        cols = pl.ds(pl.multiple_of(h * GW, GW), GW)
        return [
            pltpu.make_async_copy(wq_hbm.at[:, cols], wqbuf.at[s], a_sem.at[s, 0]),
            pltpu.make_async_copy(k_hbm.at[h], kbuf.at[s], a_sem.at[s, 1]),
            pltpu.make_async_copy(v_hbm.at[h], vbuf.at[s], a_sem.at[s, 2]),
            pltpu.make_async_copy(wot_hbm.at[:, cols], wobuf.at[h % 3], a_sem.at[s, 3]),
        ]

    def moe_copies(j, s):
        cols = pl.ds(pl.multiple_of(j * FC, 128), FC)
        return [
            pltpu.make_async_copy(wg_hbm.at[:, cols], wgbuf.at[s], m_sem.at[s, 0]),
            pltpu.make_async_copy(wu_hbm.at[:, cols], wubuf.at[s], m_sem.at[s, 1]),
            pltpu.make_async_copy(wdt_hbm.at[:, cols], wdbuf.at[s], m_sem.at[s, 2]),
        ]

    @pl.when(g == 0)
    def _prologue():
        wr_copy().start()
        for c in range(XDEPTH):
            x_copy(c).start()
        wr_copy().wait()
        wr = jnp.broadcast_to(wr_ref[...].reshape(1, D), (8, D))
        rs = []
        for c in range(NCH):
            cols = pl.ds(c * TQ, TQ)
            x_copy(c).wait()
            if c + XDEPTH < NCH:
                x_copy(c + XDEPTH).start()
            if c == NCH - 3:
                for cp in attn_copies(0, 0):
                    cp.start()
            x = xt_ref[:, cols].astype(_F32)
            d = x - x[0:1, :]
            md = jnp.sum(d, axis=0, keepdims=True) * (1.0 / D)
            var = jnp.sum(d * d, axis=0, keepdims=True) * (1.0 / D) - md * md
            var = jnp.maximum(var, 0.0)
            mean = x[0:1, :] + md
            den = _rb(jnp.sqrt(_rb(_rb(var) + EPS)))
            xn32 = _rb(x - _rb(mean)) * _recip(den)
            xn = xn32.astype(_BF16)
            xnt_ref[:, cols] = xn
            xn_ref[cols, :] = xn32.T.astype(_BF16)
            rs.append(jnp.dot(wr, xn, preferred_element_type=_F32)[0:1, :])
        r = _rb(jnp.concatenate(rs, axis=1)) + 0.0
        pos = jax.lax.broadcasted_iota(_I32, (1, S), 1)
        bits = pltpu.bitcast(r, _I32)
        key = jnp.where(bits < 0, bits ^ 0x7FFF0000, bits) | (S - 1 - pos)
        row16 = jax.lax.broadcasted_iota(_I32, (16, D), 0)
        sels, rsel, xsel = [], [], []
        for c in range(C):
            m = jnp.max(key, axis=1, keepdims=True)
            hit = key == m
            sels.append(hit.astype(_F32))
            hi = jnp.broadcast_to(m, (1, 128)) & jnp.int32(-65536)
            rsel.append(pltpu.bitcast(jnp.where(hi < 0, hi ^ 0x7FFF0000, hi), _F32))
            key = jnp.where(hit, jnp.iinfo(jnp.int32).min, key)
            idx = (S - 1) - (m[0, 0] & (S - 1))
            blk = xn_ref[pl.ds(pl.multiple_of((idx // 16) * 16, 16), 16), :].astype(_F32)
            xsel.append(jnp.sum(jnp.where(row16 == idx % 16, blk, 0.0), axis=0, keepdims=True))
        sel_ref[...] = jnp.concatenate(
            sels + [jnp.zeros((CP - C, S), _F32)], axis=0).astype(_BF16)
        rsel_ref[...] = jnp.concatenate(rsel + [jnp.zeros((CP - C, 128), _F32)], axis=0)
        xsel_ref[...] = jnp.concatenate(
            xsel + [jnp.zeros((CP - C, D), _F32)], axis=0).astype(_BF16)
        y_ref[...] = jnp.zeros_like(y_ref)
        wobuf[2] = jnp.zeros((D, GW), _BF16)
        for h in range(REP):
            raw_ref[h, 0] = jnp.zeros((TQ, 128), _F32)
            raw_ref[h, 1] = jnp.ones((TQ, 128), _F32)

    moe_active = jnp.logical_and(g >= 1, g <= NF)

    @pl.when(moe_active)
    def _moe_wait():
        for cp in moe_copies(g - 1, slot):
            cp.wait()

    for cp in attn_copies(g, slot):
        cp.wait()

    @pl.when(g + 1 < HKV)
    def _prefetch_attn():
        for cp in attn_copies(g + 1, 1 - slot):
            cp.start()

    @pl.when(g < NF)
    def _prefetch_moe():
        for cp in moe_copies(g, 1 - slot):
            cp.start()


    k = kbuf[slot]
    v = vbuf[slot]

    def qproj(c):
        q = jnp.dot(xn_ref[pl.ds(c * TQ, TQ), :], wqbuf[slot], preferred_element_type=_F32)
        return (q * QSCALE).astype(_BF16)

    def qk(q, h):
        return jax.lax.dot_general(q[:, h * DH:(h + 1) * DH], k, _NT, preferred_element_type=_F32)

    def normalize(o, part):
        l = jnp.sum(part, axis=-1, keepdims=True)
        return (o * _recip(l)).astype(_BF16)

    def pv(s):
        m = jnp.max(_tree(s, jnp.maximum), axis=-1, keepdims=True)
        p = jnp.exp2(s - m)
        tiles = [p[:, i * 128:(i + 1) * 128] for i in range(S // 128)]
        acc = None
        for g0 in range(0, len(tiles), 4):
            t = (tiles[g0] + tiles[g0 + 1]) + (tiles[g0 + 2] + tiles[g0 + 3])
            acc = t if acc is None else acc + t
            tiles[g0 + 3] = jnp.minimum(tiles[g0 + 3], acc)
        pb = jnp.concatenate(tiles, axis=-1).astype(_BF16)
        return jnp.dot(pb, v, preferred_element_type=_F32), acc

    def oproj(c, oa, ob, wo, first):
        o2 = jnp.concatenate([oa, ob], axis=-1)
        cols = pl.ds(c * TQ, TQ)
        prev = acc_ref[:, cols]
        if first:
            prev = jnp.where(g > 0, prev, 0.0)
        acc_ref[:, cols] = prev + jax.lax.dot_general(
            wo, o2, _NT, preferred_element_type=_F32)

    def deferred_oproj(wo, first):
        oa = normalize(raw_ref[0, 0], raw_ref[0, 1])
        ob = normalize(raw_ref[1, 0], raw_ref[1, 1])
        oproj(NCH - 1, oa, ob, wo, first)

    KT = [(k0, min(k0 + 128, D)) for k0 in range(0, D, 128)]
    xs = xsel_ref[...]

    def up_piece(wbuf, i):
        k0, k1 = KT[i]
        return jnp.dot(xs[:, k0:k1], wbuf[slot, k0:k1, :], preferred_element_type=_F32)

    def down_piece(hb, i):
        return jax.lax.dot_general(hb[:, i * 128:(i + 1) * 128],
                                   wdbuf[slot, :, i * 128:(i + 1) * 128], _NT,
                                   preferred_element_type=_F32)

    pieces = [(wgbuf, i) for i in range(len(KT))] + [(wubuf, i) for i in range(len(KT))]
    parts = []
    qs = []
    for c in range(NCH):
        qs.append(qproj(c))
        parts.append(up_piece(*pieces[c]))
    deferred_oproj(wobuf[(g + 2) % 3], True)
    parts.append(up_piece(*pieces[NCH]))
    outs = []
    hb = None
    ys = []
    for c in range(NCH):
        sa = qk(qs[c], 0)
        if c == 0:
            parts.append(up_piece(*pieces[NCH + 1]))
            gate = sum(parts[1:len(KT)], parts[0])
            up = sum(parts[len(KT) + 1:], parts[len(KT)])
            hb = ((gate * jax.nn.sigmoid(gate)) * up).astype(_BF16)
        sb = qk(qs[c], 1)
        ra, rb_ = pv(sa), pv(sb)
        if 1 <= c <= FC // 128:
            ys.append(down_piece(hb, c - 1))
        if c < NCH - 1:
            outs.append((normalize(*ra), normalize(*rb_)))
        else:
            for h, r in enumerate((ra, rb_)):
                raw_ref[h, 0] = r[0]
                raw_ref[h, 1] = r[1]
    y_ref[...] += jnp.where(moe_active, sum(ys[1:], ys[0]), 0.0)
    wo_cur = wobuf[g % 3]
    for c in range(NCH - 1):
        oproj(c, *outs[c], wo_cur, True)

    @pl.when(g == HKV - 1)
    def _epilogue():
        y = y_ref[...] * jax.nn.sigmoid(rsel_ref[:, 0:1])
        yt = jnp.concatenate([y, jnp.zeros((128 - CP, D), _F32)], axis=0).T
        yt = yt.astype(_BF16)
        for c in range(NCH):
            cols = pl.ds(c * TQ, TQ)
            if c == NCH - 1:
                deferred_oproj(wobuf[(HKV - 1) % 3], False)
            selc = jnp.concatenate(
                [sel_ref[:, cols], jnp.zeros((128 - CP, TQ), _BF16)], axis=0)
            upd = jnp.dot(yt, selc, preferred_element_type=_F32)
            hb = 0.5 * (xnt_ref[:, cols].astype(_F32) + upd)
            gate = hb + hb * jnp.tanh(hb)
            obuf[:, cols] = (xt_ref[:, cols].astype(_F32)
                             + acc_ref[:, cols] * gate).astype(_BF16)
            out_copy(c).start()
        for c in range(NCH):
            out_copy(c).wait()


@jax.jit
def pallas_recurrent_scan__gqa_block_cached__moe_arch_mod__prompt_kernel(
    A_x: jax.Array,
    A_k_cache: jax.Array,
    A_v_cache: jax.Array,
    A_wq: jax.Array,
    A_wo: jax.Array,
    B_x: jax.Array,
    B_w_r: jax.Array,
    B_w_gate: jax.Array,
    B_w_up: jax.Array,
    B_w_down: jax.Array,
):
    xt = A_x.reshape(S, D).T
    k = A_k_cache.reshape(HKV, S, DH)
    v = A_v_cache.reshape(HKV, S, DH)
    wot = A_wo.T
    wdt = B_w_down.T

    out_t = pl.pallas_call(
        _kernel,
        grid=(HKV,),
        in_specs=[pl.BlockSpec(memory_space=pl.ANY)] * 9,
        out_specs=pl.BlockSpec(memory_space=pl.ANY),
        out_shape=jax.ShapeDtypeStruct((D, S), A_x.dtype),
        scratch_shapes=[
            pltpu.VMEM((D, S), _BF16),
            pltpu.VMEM((D,), _BF16),
            pltpu.VMEM((2, S, DH), _BF16),
            pltpu.VMEM((2, S, DH), _BF16),
            pltpu.VMEM((2, D, GW), _BF16),
            pltpu.VMEM((3, D, GW), _BF16),
            pltpu.VMEM((2, D, FC), _BF16),
            pltpu.VMEM((2, D, FC), _BF16),
            pltpu.VMEM((2, D, FC), _BF16),
            pltpu.VMEM((D, S), _BF16),
            pltpu.VMEM((S, D), _BF16),
            pltpu.VMEM((D, S), _BF16),
            pltpu.VMEM((D, S), _F32),
            pltpu.VMEM((CP, S), _BF16),
            pltpu.VMEM((CP, D), _BF16),
            pltpu.VMEM((CP, 128), _F32),
            pltpu.VMEM((CP, D), _F32),
            pltpu.VMEM((REP, 2, TQ, 128), _F32),
            pltpu.SemaphoreType.DMA((NCH,)),
            pltpu.SemaphoreType.DMA((NCH,)),
            pltpu.SemaphoreType.DMA((1,)),
            pltpu.SemaphoreType.DMA((2, 4)),
            pltpu.SemaphoreType.DMA((2, 3)),
        ],
        compiler_params=pltpu.CompilerParams(
            dimension_semantics=("arbitrary",),
            vmem_limit_bytes=126 * 1024 * 1024,
            disable_bounds_checks=True,
        ),
        name="fused_gqa_mod",
    )(xt, k, v, A_wq, wot, B_w_r, B_w_gate, B_w_up, wdt)
    return out_t.T.reshape(1, S, D)
```

```python
import math

import jax
import jax.numpy as jnp
import jax.experimental.pallas as pl
import jax.experimental.pallas.tpu as pltpu

_BF16 = jnp.bfloat16
_F32 = jnp.float32
_I32 = jnp.int32

S = 2048
D = 576
HQ = 32
HKV = 16
DH = 128
REP = HQ // HKV
GW = REP * DH
F = 4608
C = 8
CP = 16
EPS = 1e-5

TQ = 256
NCH = S // TQ
FC = 384
NF = F // FC
XDEPTH = 2
QSCALE = (DH ** -0.5) * math.log2(math.e)

_NT = (((1,), (1,)), ((), ()))


def _rb(x):
    return x.astype(_BF16).astype(_F32)


def _recip(x):
    r = pl.reciprocal(x, approx=True)
    return r * (2.0 - x * r)


def _tree(a, op):
    tiles = [a[:, i * 128:(i + 1) * 128] for i in range(a.shape[1] // 128)]
    while len(tiles) > 1:
        tiles = [op(tiles[i], tiles[i + 1]) for i in range(0, len(tiles), 2)]
    return tiles[0]


def _kernel(xt_hbm, k_hbm, v_hbm, wq_hbm, wot_hbm, wr_hbm, wg_hbm, wu_hbm, wdt_hbm,
            out_hbm,
            xt_ref, wr_ref, kbuf, vbuf, wqbuf, wobuf, wgbuf, wubuf, wdbuf, obuf,
            xn_ref, xnt_ref, acc_ref, sel_ref, xsel_ref, rsel_ref, y_ref,
            raw_ref, x_sem, o_sem, w_sem, a_sem, m_sem):
    g = pl.program_id(0)
    slot = g % 2

    def x_copy(c):
        cols = pl.ds(c * TQ, TQ)
        return pltpu.make_async_copy(xt_hbm.at[:, cols], xt_ref.at[:, cols], x_sem.at[c])

    def out_copy(c):
        cols = pl.ds(c * TQ, TQ)
        return pltpu.make_async_copy(obuf.at[:, cols], out_hbm.at[:, cols], o_sem.at[c])

    def wr_copy():
        return pltpu.make_async_copy(wr_hbm, wr_ref, w_sem.at[0])

    def attn_copies(h, s):
        cols = pl.ds(pl.multiple_of(h * GW, GW), GW)
        return [
            pltpu.make_async_copy(wq_hbm.at[:, cols], wqbuf.at[s], a_sem.at[s, 0]),
            pltpu.make_async_copy(k_hbm.at[h], kbuf.at[s], a_sem.at[s, 1]),
            pltpu.make_async_copy(v_hbm.at[h], vbuf.at[s], a_sem.at[s, 2]),
            pltpu.make_async_copy(wot_hbm.at[:, cols], wobuf.at[h % 3], a_sem.at[s, 3]),
        ]

    def moe_copies(j, s):
        cols = pl.ds(pl.multiple_of(j * FC, 128), FC)
        return [
            pltpu.make_async_copy(wg_hbm.at[:, cols], wgbuf.at[s], m_sem.at[s, 0]),
            pltpu.make_async_copy(wu_hbm.at[:, cols], wubuf.at[s], m_sem.at[s, 1]),
            pltpu.make_async_copy(wdt_hbm.at[:, cols], wdbuf.at[s], m_sem.at[s, 2]),
        ]

    @pl.when(g == 0)
    def _prologue():
        wr_copy().start()
        for c in range(XDEPTH):
            x_copy(c).start()
        wr_copy().wait()
        wr = jnp.broadcast_to(wr_ref[...].reshape(1, D), (8, D))
        rs = []
        for c in range(NCH):
            cols = pl.ds(c * TQ, TQ)
            x_copy(c).wait()
            if c + XDEPTH < NCH:
                x_copy(c + XDEPTH).start()
            if c == NCH - 3:
                for cp in attn_copies(0, 0):
                    cp.start()
            x0 = xt_ref[0:16, cols].astype(_F32)[0:1, :]
            s1 = s2 = None
            for r0 in range(0, D, 16):
                d = xt_ref[r0:r0 + 16, cols].astype(_F32) - x0
                s1 = d if s1 is None else s1 + d
                s2 = d * d if s2 is None else s2 + d * d
            md = jnp.sum(s1, axis=0, keepdims=True) * (1.0 / D)
            var = jnp.sum(s2, axis=0, keepdims=True) * (1.0 / D) - md * md
            var = jnp.maximum(var, 0.0)
            mean = _rb(x0 + md)
            inv = _recip(_rb(jnp.sqrt(_rb(_rb(var) + EPS))))
            xn32 = jnp.concatenate(
                [_rb(xt_ref[r0:r0 + 64, cols].astype(_F32) - mean) * inv
                 for r0 in range(0, D, 64)], axis=0)
            xn = xn32.astype(_BF16)
            xnt_ref[:, cols] = xn
            xn_ref[cols, :] = xn32.T.astype(_BF16)
            rs.append(jnp.dot(wr, xn, preferred_element_type=_F32)[0:1, :])
        r = _rb(jnp.concatenate(rs, axis=1)) + 0.0
        pos = jax.lax.broadcasted_iota(_I32, (1, S), 1)
        bits = pltpu.bitcast(r, _I32)
        key = jnp.where(bits < 0, bits ^ 0x7FFF0000, bits) | (S - 1 - pos)
        row16 = jax.lax.broadcasted_iota(_I32, (16, D), 0)
        sels, rsel, xsel = [], [], []
        for c in range(C):
            m = jnp.max(key, axis=1, keepdims=True)
            hit = key == m
            sels.append(hit.astype(_F32))
            hi = jnp.broadcast_to(m, (1, 128)) & jnp.int32(-65536)
            rsel.append(pltpu.bitcast(jnp.where(hi < 0, hi ^ 0x7FFF0000, hi), _F32))
            key = jnp.where(hit, jnp.iinfo(jnp.int32).min, key)
            idx = (S - 1) - (m[0, 0] & (S - 1))
            blk = xn_ref[pl.ds(pl.multiple_of((idx // 16) * 16, 16), 16), :].astype(_F32)
            xsel.append(jnp.sum(jnp.where(row16 == idx % 16, blk, 0.0), axis=0, keepdims=True))
        sel_ref[...] = jnp.concatenate(
            sels + [jnp.zeros((CP - C, S), _F32)], axis=0).astype(_BF16)
        rsel_ref[...] = jnp.concatenate(rsel + [jnp.zeros((CP - C, 128), _F32)], axis=0)
        xsel_ref[...] = jnp.concatenate(
            xsel + [jnp.zeros((CP - C, D), _F32)], axis=0).astype(_BF16)
        y_ref[...] = jnp.zeros_like(y_ref)
        wobuf[2] = jnp.zeros((D, GW), _BF16)
        for h in range(REP):
            raw_ref[h, 0] = jnp.zeros((TQ, 128), _F32)
            raw_ref[h, 1] = jnp.ones((TQ, 128), _F32)

    moe_active = jnp.logical_and(g >= 1, g <= NF)

    @pl.when(moe_active)
    def _moe_wait():
        for cp in moe_copies(g - 1, slot):
            cp.wait()

    for cp in attn_copies(g, slot):
        cp.wait()

    @pl.when(g + 1 < HKV)
    def _prefetch_attn():
        for cp in attn_copies(g + 1, 1 - slot):
            cp.start()

    @pl.when(g < NF)
    def _prefetch_moe():
        for cp in moe_copies(g, 1 - slot):
            cp.start()


    k = kbuf[slot]
    v = vbuf[slot]

    def qproj(c):
        q = jnp.dot(xn_ref[pl.ds(c * TQ, TQ), :], wqbuf[slot], preferred_element_type=_F32)
        return (q * QSCALE).astype(_BF16)

    def qk(q, h):
        return jax.lax.dot_general(q[:, h * DH:(h + 1) * DH], k, _NT, preferred_element_type=_F32)

    def normalize(o, part):
        l = jnp.sum(part, axis=-1, keepdims=True)
        return (o * _recip(l)).astype(_BF16)

    def pv(s):
        m = jnp.max(_tree(s, jnp.maximum), axis=-1, keepdims=True)
        p = jnp.exp2(s - m)
        tiles = [p[:, i * 128:(i + 1) * 128] for i in range(S // 128)]
        acc = None
        for g0 in range(0, len(tiles), 4):
            t = (tiles[g0] + tiles[g0 + 1]) + (tiles[g0 + 2] + tiles[g0 + 3])
            acc = t if acc is None else acc + t
            tiles[g0 + 3] = jnp.minimum(tiles[g0 + 3], acc)
        pb = jnp.concatenate(tiles, axis=-1).astype(_BF16)
        return jnp.dot(pb, v, preferred_element_type=_F32), acc

    def oproj(c, oa, ob, wo, first):
        o2 = jnp.concatenate([oa, ob], axis=-1)
        cols = pl.ds(c * TQ, TQ)
        prev = acc_ref[:, cols]
        if first:
            prev = jnp.where(g > 0, prev, 0.0)
        acc_ref[:, cols] = prev + jax.lax.dot_general(
            wo, o2, _NT, preferred_element_type=_F32)

    def deferred_oproj(wo, first):
        oa = normalize(raw_ref[0, 0], raw_ref[0, 1])
        ob = normalize(raw_ref[1, 0], raw_ref[1, 1])
        oproj(NCH - 1, oa, ob, wo, first)

    KT = [(k0, min(k0 + 128, D)) for k0 in range(0, D, 128)]
    xs = xsel_ref[...]

    def up_piece(wbuf, i):
        k0, k1 = KT[i]
        return jnp.dot(xs[:, k0:k1], wbuf[slot, k0:k1, :], preferred_element_type=_F32)

    def down_piece(hb, i):
        return jax.lax.dot_general(hb[:, i * 128:(i + 1) * 128],
                                   wdbuf[slot, :, i * 128:(i + 1) * 128], _NT,
                                   preferred_element_type=_F32)

    pieces = [(wgbuf, i) for i in range(len(KT))] + [(wubuf, i) for i in range(len(KT))]
    parts = []
    qs = []
    for c in range(NCH):
        qs.append(qproj(c))
        parts.append(up_piece(*pieces[c]))
    deferred_oproj(wobuf[(g + 2) % 3], True)
    parts.append(up_piece(*pieces[NCH]))
    outs = []
    hb = None
    ys = []
    for c in range(NCH):
        sa = qk(qs[c], 0)
        if c == 0:
            parts.append(up_piece(*pieces[NCH + 1]))
            gate = sum(parts[1:len(KT)], parts[0])
            up = sum(parts[len(KT) + 1:], parts[len(KT)])
            hb = ((gate * jax.nn.sigmoid(gate)) * up).astype(_BF16)
        sb = qk(qs[c], 1)
        ra, rb_ = pv(sa), pv(sb)
        if 1 <= c <= FC // 128:
            ys.append(down_piece(hb, c - 1))
        if c < NCH - 1:
            outs.append((normalize(*ra), normalize(*rb_)))
        else:
            for h, r in enumerate((ra, rb_)):
                raw_ref[h, 0] = r[0]
                raw_ref[h, 1] = r[1]
    y_ref[...] += jnp.where(moe_active, sum(ys[1:], ys[0]), 0.0)
    wo_cur = wobuf[g % 3]
    for c in range(NCH - 1):
        oproj(c, *outs[c], wo_cur, True)

    @pl.when(g == HKV - 1)
    def _epilogue():
        y = y_ref[...] * jax.nn.sigmoid(rsel_ref[:, 0:1])
        yt = jnp.concatenate([y, jnp.zeros((128 - CP, D), _F32)], axis=0).T
        yt = yt.astype(_BF16)
        for c in range(NCH):
            cols = pl.ds(c * TQ, TQ)
            if c == NCH - 1:
                deferred_oproj(wobuf[(HKV - 1) % 3], False)
            selc = jnp.concatenate(
                [sel_ref[:, cols], jnp.zeros((128 - CP, TQ), _BF16)], axis=0)
            upd = jnp.dot(yt, selc, preferred_element_type=_F32)
            hb = 0.5 * (xnt_ref[:, cols].astype(_F32) + upd)
            gate = hb + hb * jnp.tanh(hb)
            obuf[:, cols] = (xt_ref[:, cols].astype(_F32)
                             + acc_ref[:, cols] * gate).astype(_BF16)
            out_copy(c).start()
        for c in range(NCH):
            out_copy(c).wait()


@jax.jit
def pallas_recurrent_scan__gqa_block_cached__moe_arch_mod__prompt_kernel(
    A_x: jax.Array,
    A_k_cache: jax.Array,
    A_v_cache: jax.Array,
    A_wq: jax.Array,
    A_wo: jax.Array,
    B_x: jax.Array,
    B_w_r: jax.Array,
    B_w_gate: jax.Array,
    B_w_up: jax.Array,
    B_w_down: jax.Array,
):
    xt = A_x.reshape(S, D).T
    k = A_k_cache.reshape(HKV, S, DH)
    v = A_v_cache.reshape(HKV, S, DH)
    wot = A_wo.T
    wdt = B_w_down.T

    out_t = pl.pallas_call(
        _kernel,
        grid=(HKV,),
        in_specs=[pl.BlockSpec(memory_space=pl.ANY)] * 9,
        out_specs=pl.BlockSpec(memory_space=pl.ANY),
        out_shape=jax.ShapeDtypeStruct((D, S), A_x.dtype),
        scratch_shapes=[
            pltpu.VMEM((D, S), _BF16),
            pltpu.VMEM((D,), _BF16),
            pltpu.VMEM((2, S, DH), _BF16),
            pltpu.VMEM((2, S, DH), _BF16),
            pltpu.VMEM((2, D, GW), _BF16),
            pltpu.VMEM((3, D, GW), _BF16),
            pltpu.VMEM((2, D, FC), _BF16),
            pltpu.VMEM((2, D, FC), _BF16),
            pltpu.VMEM((2, D, FC), _BF16),
            pltpu.VMEM((D, S), _BF16),
            pltpu.VMEM((S, D), _BF16),
            pltpu.VMEM((D, S), _BF16),
            pltpu.VMEM((D, S), _F32),
            pltpu.VMEM((CP, S), _BF16),
            pltpu.VMEM((CP, D), _BF16),
            pltpu.VMEM((CP, 128), _F32),
            pltpu.VMEM((CP, D), _F32),
            pltpu.VMEM((REP, 2, TQ, 128), _F32),
            pltpu.SemaphoreType.DMA((NCH,)),
            pltpu.SemaphoreType.DMA((NCH,)),
            pltpu.SemaphoreType.DMA((1,)),
            pltpu.SemaphoreType.DMA((2, 4)),
            pltpu.SemaphoreType.DMA((2, 3)),
        ],
        compiler_params=pltpu.CompilerParams(
            dimension_semantics=("arbitrary",),
            vmem_limit_bytes=126 * 1024 * 1024,
            disable_bounds_checks=True,
        ),
        name="fused_gqa_mod",
    )(xt, k, v, A_wq, wot, B_w_r, B_w_gate, B_w_up, wdt)
    return out_t.T.reshape(1, S, D)
```

```python
import math

import jax
import jax.numpy as jnp
import jax.experimental.pallas as pl
import jax.experimental.pallas.tpu as pltpu

_BF16 = jnp.bfloat16
_F32 = jnp.float32
_I32 = jnp.int32

S = 2048
D = 576
HQ = 32
HKV = 16
DH = 128
REP = HQ // HKV
GW = REP * DH
F = 4608
C = 8
CP = 16
EPS = 1e-5

TQ = 256
NCH = S // TQ
FC = 384
NF = F // FC
XDEPTH = 2
QSCALE = (DH ** -0.5) * math.log2(math.e)

_NT = (((1,), (1,)), ((), ()))


def _rb(x):
    return x.astype(_BF16).astype(_F32)


def _recip(x):
    r = pl.reciprocal(x, approx=True)
    return r * (2.0 - x * r)


def _tree(a, op):
    tiles = [a[:, i * 128:(i + 1) * 128] for i in range(a.shape[1] // 128)]
    while len(tiles) > 1:
        tiles = [op(tiles[i], tiles[i + 1]) for i in range(0, len(tiles), 2)]
    return tiles[0]


def _kernel(xt_hbm, k_hbm, v_hbm, wq_hbm, wot_hbm, wr_hbm, wg_hbm, wu_hbm, wdt_hbm,
            out_hbm,
            xt_ref, wr_ref, kbuf, vbuf, wqbuf, wobuf, wgbuf, wubuf, wdbuf, obuf,
            xn_ref, xnt_ref, acc_ref, sel_ref, xsel_ref, rsel_ref, y_ref,
            raw_ref, q_ref, hb_ref, x_sem, o_sem, w_sem, a_sem, m_sem):
    g = pl.program_id(0)
    slot = g % 2

    def x_copy(c):
        cols = pl.ds(c * TQ, TQ)
        return pltpu.make_async_copy(xt_hbm.at[:, cols], xt_ref.at[:, cols], x_sem.at[c])

    def out_copy(c):
        cols = pl.ds(c * TQ, TQ)
        return pltpu.make_async_copy(obuf.at[:, cols], out_hbm.at[:, cols], o_sem.at[c])

    def wr_copy():
        return pltpu.make_async_copy(wr_hbm, wr_ref, w_sem.at[0])

    def attn_copies(h, s):
        cols = pl.ds(pl.multiple_of(h * GW, GW), GW)
        return [
            pltpu.make_async_copy(wq_hbm.at[:, cols], wqbuf.at[s], a_sem.at[s, 0]),
            pltpu.make_async_copy(k_hbm.at[h], kbuf.at[s], a_sem.at[s, 1]),
            pltpu.make_async_copy(v_hbm.at[h], vbuf.at[s], a_sem.at[s, 2]),
            pltpu.make_async_copy(wot_hbm.at[:, cols], wobuf.at[h % 3], a_sem.at[s, 3]),
        ]

    def moe_copies(j, s):
        cols = pl.ds(pl.multiple_of(j * FC, 128), FC)
        return [
            pltpu.make_async_copy(wg_hbm.at[:, cols], wgbuf.at[s], m_sem.at[s, 0]),
            pltpu.make_async_copy(wu_hbm.at[:, cols], wubuf.at[s], m_sem.at[s, 1]),
            pltpu.make_async_copy(wdt_hbm.at[:, cols], wdbuf.at[s], m_sem.at[s, 2]),
        ]

    def qproj(c):
        q = jnp.dot(xn_ref[pl.ds(c * TQ, TQ), :], wqbuf[slot], preferred_element_type=_F32)
        q_ref[c] = (q * QSCALE).astype(_BF16)

    def normalize(o, part):
        l = jnp.sum(part, axis=-1, keepdims=True)
        return (o * _recip(l)).astype(_BF16)

    def oproj(c, oa, ob, wo, nheads_done):
        o2 = jnp.concatenate([oa, ob], axis=-1)
        cols = pl.ds(c * TQ, TQ)
        prev = acc_ref[:, cols]
        if nheads_done is not None:
            prev = jnp.where(nheads_done > 0, prev, 0.0)
        acc_ref[:, cols] = prev + jax.lax.dot_general(
            wo, o2, _NT, preferred_element_type=_F32)

    def deferred_oproj(wo, nheads_done):
        oa = normalize(raw_ref[0, 0], raw_ref[0, 1])
        ob = normalize(raw_ref[1, 0], raw_ref[1, 1])
        oproj(NCH - 1, oa, ob, wo, nheads_done)

    @pl.when(g == 0)
    def _prologue():
        first = attn_copies(0, 0)
        wr_copy().start()
        for c in range(XDEPTH):
            x_copy(c).start()
        first[0].start()
        wr_copy().wait()
        wr = jnp.broadcast_to(wr_ref[...].reshape(1, D), (8, D))
        rs = []
        for c in range(NCH):
            cols = pl.ds(c * TQ, TQ)
            x_copy(c).wait()
            if c + XDEPTH < NCH:
                x_copy(c + XDEPTH).start()
            if c == NCH - 3:
                for cp in first[1:]:
                    cp.start()
            if c == 1:
                first[0].wait()
            x0 = xt_ref[0:16, cols].astype(_F32)[0:1, :]
            s1 = s2 = None
            for r0 in range(0, D, 16):
                d = xt_ref[r0:r0 + 16, cols].astype(_F32) - x0
                s1 = d if s1 is None else s1 + d
                s2 = d * d if s2 is None else s2 + d * d
            md = jnp.sum(s1, axis=0, keepdims=True) * (1.0 / D)
            var = jnp.sum(s2, axis=0, keepdims=True) * (1.0 / D) - md * md
            var = jnp.maximum(var, 0.0)
            mean = _rb(x0 + md)
            inv = _recip(_rb(jnp.sqrt(_rb(_rb(var) + EPS))))
            if c >= 1:
                qproj(c - 1)
            xn32 = jnp.concatenate(
                [_rb(xt_ref[r0:r0 + 64, cols].astype(_F32) - mean) * inv
                 for r0 in range(0, D, 64)], axis=0)
            xn = xn32.astype(_BF16)
            xnt_ref[:, cols] = xn
            xn_ref[cols, :] = xn32.T.astype(_BF16)
            rs.append(jnp.dot(wr, xn, preferred_element_type=_F32)[0:1, :])
        qproj(NCH - 1)
        r = _rb(jnp.concatenate(rs, axis=1)) + 0.0
        pos = jax.lax.broadcasted_iota(_I32, (1, S), 1)
        bits = pltpu.bitcast(r, _I32)
        key = jnp.where(bits < 0, bits ^ 0x7FFF0000, bits) | (S - 1 - pos)
        row16 = jax.lax.broadcasted_iota(_I32, (16, D), 0)
        sels, rsel, xsel = [], [], []
        for c in range(C):
            m = jnp.max(key, axis=1, keepdims=True)
            hit = key == m
            sels.append(hit.astype(_F32))
            hi = jnp.broadcast_to(m, (1, 128)) & jnp.int32(-65536)
            rsel.append(pltpu.bitcast(jnp.where(hi < 0, hi ^ 0x7FFF0000, hi), _F32))
            key = jnp.where(hit, jnp.iinfo(jnp.int32).min, key)
            idx = (S - 1) - (m[0, 0] & (S - 1))
            blk = xn_ref[pl.ds(pl.multiple_of((idx // 16) * 16, 16), 16), :].astype(_F32)
            xsel.append(jnp.sum(jnp.where(row16 == idx % 16, blk, 0.0), axis=0, keepdims=True))
        sel_ref[...] = jnp.concatenate(
            sels + [jnp.zeros((CP - C, S), _F32)], axis=0).astype(_BF16)
        rsel_ref[...] = jnp.concatenate(rsel + [jnp.zeros((CP - C, 128), _F32)], axis=0)
        xsel_ref[...] = jnp.concatenate(
            xsel + [jnp.zeros((CP - C, D), _F32)], axis=0).astype(_BF16)
        y_ref[...] = jnp.zeros_like(y_ref)
        hb_ref[...] = jnp.zeros_like(hb_ref)

    moe_active = jnp.logical_and(g >= 1, g <= NF)
    cur = attn_copies(g, slot)
    KT = [(k0, min(k0 + 128, D)) for k0 in range(0, D, 128)]

    @pl.when(moe_active)
    def _moe_wait():
        for cp in moe_copies(g - 1, slot):
            cp.wait()

    @pl.when(g >= 1)
    def _project():
        cur[0].wait()
        xs = xsel_ref[...]

        def up_piece(wbuf, i):
            k0, k1 = KT[i]
            return jnp.dot(xs[:, k0:k1], wbuf[slot, k0:k1, :], preferred_element_type=_F32)

        pieces = [(wgbuf, i) for i in range(len(KT))] + [(wubuf, i) for i in range(len(KT))]
        parts = []
        for c in range(NCH):
            qproj(c)
            parts.append(up_piece(*pieces[c]))
            if c >= NCH - 2:
                parts.append(up_piece(*pieces[c + 2]))
        deferred_oproj(wobuf[(g + 2) % 3], g - 1)
        gate = sum(parts[1:len(KT)], parts[0])
        up = sum(parts[len(KT) + 1:], parts[len(KT)])
        hb_ref[...] = ((gate * jax.nn.sigmoid(gate)) * up).astype(_BF16)

    for cp in cur[1:]:
        cp.wait()

    @pl.when(g + 1 < HKV)
    def _prefetch_attn():
        for cp in attn_copies(g + 1, 1 - slot):
            cp.start()

    @pl.when(g < NF)
    def _prefetch_moe():
        for cp in moe_copies(g, 1 - slot):
            cp.start()


    k = kbuf[slot]
    v = vbuf[slot]

    def qk(c, h):
        return jax.lax.dot_general(q_ref[c, :, h * DH:(h + 1) * DH], k, _NT,
                                   preferred_element_type=_F32)

    def pv(s):
        m = jnp.max(_tree(s, jnp.maximum), axis=-1, keepdims=True)
        p = jnp.exp2(s - m)
        tiles = [p[:, i * 128:(i + 1) * 128] for i in range(S // 128)]
        acc = None
        for g0 in range(0, len(tiles), 4):
            t = (tiles[g0] + tiles[g0 + 1]) + (tiles[g0 + 2] + tiles[g0 + 3])
            acc = t if acc is None else acc + t
            tiles[g0 + 3] = jnp.minimum(tiles[g0 + 3], acc)
        pb = jnp.concatenate(tiles, axis=-1).astype(_BF16)
        return jnp.dot(pb, v, preferred_element_type=_F32), acc

    hb = hb_ref[...]

    def down_piece(i):
        return jax.lax.dot_general(hb[:, i * 128:(i + 1) * 128],
                                   wdbuf[slot, :, i * 128:(i + 1) * 128], _NT,
                                   preferred_element_type=_F32)

    outs = []
    ys = []
    for c in range(NCH):
        sa = qk(c, 0)
        sb = qk(c, 1)
        ra, rb_ = pv(sa), pv(sb)
        if c < FC // 128:
            ys.append(down_piece(c))
        if c < NCH - 1:
            outs.append((normalize(*ra), normalize(*rb_)))
        else:
            for h, r in enumerate((ra, rb_)):
                raw_ref[h, 0] = r[0]
                raw_ref[h, 1] = r[1]
    y_ref[...] += jnp.where(moe_active, sum(ys[1:], ys[0]), 0.0)
    wo_cur = wobuf[g % 3]
    for c in range(NCH - 1):
        oproj(c, *outs[c], wo_cur, g)

    @pl.when(g == HKV - 1)
    def _epilogue():
        y = y_ref[...] * jax.nn.sigmoid(rsel_ref[:, 0:1])
        yt = jnp.concatenate([y, jnp.zeros((128 - CP, D), _F32)], axis=0).T
        yt = yt.astype(_BF16)
        for c in range(NCH):
            cols = pl.ds(c * TQ, TQ)
            if c == NCH - 1:
                deferred_oproj(wobuf[(HKV - 1) % 3], None)
            selc = jnp.concatenate(
                [sel_ref[:, cols], jnp.zeros((128 - CP, TQ), _BF16)], axis=0)
            upd = jnp.dot(yt, selc, preferred_element_type=_F32)
            hb = 0.5 * (xnt_ref[:, cols].astype(_F32) + upd)
            gate = hb + hb * jnp.tanh(hb)
            obuf[:, cols] = (xt_ref[:, cols].astype(_F32)
                             + acc_ref[:, cols] * gate).astype(_BF16)
            out_copy(c).start()
        for c in range(NCH):
            out_copy(c).wait()


@jax.jit
def pallas_recurrent_scan__gqa_block_cached__moe_arch_mod__prompt_kernel(
    A_x: jax.Array,
    A_k_cache: jax.Array,
    A_v_cache: jax.Array,
    A_wq: jax.Array,
    A_wo: jax.Array,
    B_x: jax.Array,
    B_w_r: jax.Array,
    B_w_gate: jax.Array,
    B_w_up: jax.Array,
    B_w_down: jax.Array,
):
    xt = A_x.reshape(S, D).T
    k = A_k_cache.reshape(HKV, S, DH)
    v = A_v_cache.reshape(HKV, S, DH)
    wot = A_wo.T
    wdt = B_w_down.T

    out_t = pl.pallas_call(
        _kernel,
        grid=(HKV,),
        in_specs=[pl.BlockSpec(memory_space=pl.ANY)] * 9,
        out_specs=pl.BlockSpec(memory_space=pl.ANY),
        out_shape=jax.ShapeDtypeStruct((D, S), A_x.dtype),
        scratch_shapes=[
            pltpu.VMEM((D, S), _BF16),
            pltpu.VMEM((D,), _BF16),
            pltpu.VMEM((2, S, DH), _BF16),
            pltpu.VMEM((2, S, DH), _BF16),
            pltpu.VMEM((2, D, GW), _BF16),
            pltpu.VMEM((3, D, GW), _BF16),
            pltpu.VMEM((2, D, FC), _BF16),
            pltpu.VMEM((2, D, FC), _BF16),
            pltpu.VMEM((2, D, FC), _BF16),
            pltpu.VMEM((D, S), _BF16),
            pltpu.VMEM((S, D), _BF16),
            pltpu.VMEM((D, S), _BF16),
            pltpu.VMEM((D, S), _F32),
            pltpu.VMEM((CP, S), _BF16),
            pltpu.VMEM((CP, D), _BF16),
            pltpu.VMEM((CP, 128), _F32),
            pltpu.VMEM((CP, D), _F32),
            pltpu.VMEM((REP, 2, TQ, 128), _F32),
            pltpu.VMEM((NCH, TQ, GW), _BF16),
            pltpu.VMEM((CP, FC), _BF16),
            pltpu.SemaphoreType.DMA((NCH,)),
            pltpu.SemaphoreType.DMA((NCH,)),
            pltpu.SemaphoreType.DMA((1,)),
            pltpu.SemaphoreType.DMA((2, 4)),
            pltpu.SemaphoreType.DMA((2, 3)),
        ],
        compiler_params=pltpu.CompilerParams(
            dimension_semantics=("arbitrary",),
            vmem_limit_bytes=126 * 1024 * 1024,
            disable_bounds_checks=True,
        ),
        name="fused_gqa_mod",
    )(xt, k, v, A_wq, wot, B_w_r, B_w_gate, B_w_up, wdt)
    return out_t.T.reshape(1, S, D)
```

```python
import math

import jax
import jax.numpy as jnp
import jax.experimental.pallas as pl
import jax.experimental.pallas.tpu as pltpu

_BF16 = jnp.bfloat16
_F32 = jnp.float32
_I32 = jnp.int32

S = 2048
D = 576
HQ = 32
HKV = 16
DH = 128
REP = HQ // HKV
GW = REP * DH
F = 4608
C = 8
CP = 16
EPS = 1e-5

TQ = 256
NCH = S // TQ
FC = 384
NF = F // FC
XAHEAD = 2
ATT_AT = 4
XDEPTH = 2
QSCALE = (DH ** -0.5) * math.log2(math.e)

_NT = (((1,), (1,)), ((), ()))


def _rb(x):
    return x.astype(_BF16).astype(_F32)


def _recip(x):
    r = pl.reciprocal(x, approx=True)
    return r * (2.0 - x * r)


def _tree(a, op):
    tiles = [a[:, i * 128:(i + 1) * 128] for i in range(a.shape[1] // 128)]
    while len(tiles) > 1:
        tiles = [op(tiles[i], tiles[i + 1]) for i in range(0, len(tiles), 2)]
    return tiles[0]


def _kernel(xt_hbm, k_hbm, v_hbm, wq_hbm, wot_hbm, wr_hbm, wg_hbm, wu_hbm, wdt_hbm,
            out_hbm,
            xt_ref, wr_ref, kbuf, vbuf, wqbuf, wobuf, wgbuf, wubuf, wdbuf, obuf,
            xn_ref, xnt_ref, acc_ref, sel_ref, xsel_ref, rsel_ref, y_ref,
            raw_ref, q_ref, hb_ref, x_sem, o_sem, w_sem, a_sem, m_sem):
    g = pl.program_id(0)
    slot = g % 2

    def x_copy(c):
        cols = pl.ds(c * TQ, TQ)
        return pltpu.make_async_copy(xt_hbm.at[:, cols], xt_ref.at[:, cols], x_sem.at[c])

    def out_copy(c):
        cols = pl.ds(c * TQ, TQ)
        return pltpu.make_async_copy(obuf.at[:, cols], out_hbm.at[:, cols], o_sem.at[c])

    def wr_copy():
        return pltpu.make_async_copy(wr_hbm, wr_ref, w_sem.at[0])

    def attn_copies(h, s):
        cols = pl.ds(pl.multiple_of(h * GW, GW), GW)
        return [
            pltpu.make_async_copy(wq_hbm.at[:, cols], wqbuf.at[s], a_sem.at[s, 0]),
            pltpu.make_async_copy(k_hbm.at[h], kbuf.at[s], a_sem.at[s, 1]),
            pltpu.make_async_copy(v_hbm.at[h], vbuf.at[s], a_sem.at[s, 2]),
            pltpu.make_async_copy(wot_hbm.at[:, cols], wobuf.at[h % 3], a_sem.at[s, 3]),
        ]

    def moe_copies(j, s):
        cols = pl.ds(pl.multiple_of(j * FC, 128), FC)
        return [
            pltpu.make_async_copy(wg_hbm.at[:, cols], wgbuf.at[s], m_sem.at[s, 0]),
            pltpu.make_async_copy(wu_hbm.at[:, cols], wubuf.at[s], m_sem.at[s, 1]),
            pltpu.make_async_copy(wdt_hbm.at[:, cols], wdbuf.at[s], m_sem.at[s, 2]),
        ]

    def qproj(c):
        q = jnp.dot(xn_ref[pl.ds(c * TQ, TQ), :], wqbuf[slot], preferred_element_type=_F32)
        q_ref[c] = (q * QSCALE).astype(_BF16)

    def normalize(o, part):
        l = jnp.sum(part, axis=-1, keepdims=True)
        return (o * _recip(l)).astype(_BF16)

    def oproj(c, oa, ob, wo, nheads_done):
        o2 = jnp.concatenate([oa, ob], axis=-1)
        cols = pl.ds(c * TQ, TQ)
        prev = acc_ref[:, cols]
        if nheads_done is not None:
            prev = jnp.where(nheads_done > 0, prev, 0.0)
        acc_ref[:, cols] = prev + jax.lax.dot_general(
            wo, o2, _NT, preferred_element_type=_F32)

    def deferred_oproj(wo, nheads_done):
        oa = normalize(raw_ref[0, 0], raw_ref[0, 1])
        ob = normalize(raw_ref[1, 0], raw_ref[1, 1])
        oproj(NCH - 1, oa, ob, wo, nheads_done)

    @pl.when(g == 0)
    def _prologue():
        first = attn_copies(0, 0)
        wr_copy().start()
        for c in range(XDEPTH):
            x_copy(c).start()
        first[0].start()
        wr_copy().wait()
        wr = jnp.broadcast_to(wr_ref[...].reshape(1, D), (8, D))
        def layernorm(c):
            cols = pl.ds(c * TQ, TQ)
            x0 = xt_ref[0:16, cols].astype(_F32)[0:1, :]
            s1 = s2 = None
            for r0 in range(0, D, 16):
                d = xt_ref[r0:r0 + 16, cols].astype(_F32) - x0
                s1 = d if s1 is None else s1 + d
                s2 = d * d if s2 is None else s2 + d * d
            md = jnp.sum(s1, axis=0, keepdims=True) * (1.0 / D)
            var = jnp.sum(s2, axis=0, keepdims=True) * (1.0 / D) - md * md
            var = jnp.maximum(var, 0.0)
            mean = _rb(x0 + md)
            inv = _recip(_rb(jnp.sqrt(_rb(_rb(var) + EPS))))
            xn32 = jnp.concatenate(
                [_rb(xt_ref[r0:r0 + 64, cols].astype(_F32) - mean) * inv
                 for r0 in range(0, D, 64)], axis=0)
            xn = xn32.astype(_BF16)
            xnt_ref[:, cols] = xn
            xn_ref[cols, :] = xn32.T.astype(_BF16)
            return jnp.dot(wr, xn, preferred_element_type=_F32)[0:1, :]

        rs = []
        for c in range(0, NCH, 2):
            x_copy(c).wait()
            x_copy(c + 1).wait()
            for cn in (c + XAHEAD, c + XAHEAD + 1):
                if cn < NCH:
                    x_copy(cn).start()
            if c == ATT_AT:
                for cp in first[1:]:
                    cp.start()
            if c == 2:
                first[0].wait()
            if c >= 2:
                qproj(c - 2)
                qproj(c - 1)
            rs.append(layernorm(c))
            rs.append(layernorm(c + 1))
        qproj(NCH - 2)
        qproj(NCH - 1)
        r = _rb(jnp.concatenate(rs, axis=1)) + 0.0
        pos = jax.lax.broadcasted_iota(_I32, (1, S), 1)
        bits = pltpu.bitcast(r, _I32)
        key = jnp.where(bits < 0, bits ^ 0x7FFF0000, bits) | (S - 1 - pos)
        row16 = jax.lax.broadcasted_iota(_I32, (16, D), 0)
        sels, rsel, xsel = [], [], []
        for c in range(C):
            m = jnp.max(key, axis=1, keepdims=True)
            hit = key == m
            sels.append(hit.astype(_F32))
            hi = jnp.broadcast_to(m, (1, 128)) & jnp.int32(-65536)
            rsel.append(pltpu.bitcast(jnp.where(hi < 0, hi ^ 0x7FFF0000, hi), _F32))
            key = jnp.where(hit, jnp.iinfo(jnp.int32).min, key)
            idx = (S - 1) - (m[0, 0] & (S - 1))
            blk = xn_ref[pl.ds(pl.multiple_of((idx // 16) * 16, 16), 16), :].astype(_F32)
            xsel.append(jnp.sum(jnp.where(row16 == idx % 16, blk, 0.0), axis=0, keepdims=True))
        sel_ref[...] = jnp.concatenate(
            sels + [jnp.zeros((CP - C, S), _F32)], axis=0).astype(_BF16)
        rsel_ref[...] = jnp.concatenate(rsel + [jnp.zeros((CP - C, 128), _F32)], axis=0)
        xsel_ref[...] = jnp.concatenate(
            xsel + [jnp.zeros((CP - C, D), _F32)], axis=0).astype(_BF16)
        y_ref[...] = jnp.zeros_like(y_ref)
        hb_ref[...] = jnp.zeros_like(hb_ref)

    moe_active = jnp.logical_and(g >= 1, g <= NF)
    cur = attn_copies(g, slot)
    KT = [(k0, min(k0 + 128, D)) for k0 in range(0, D, 128)]

    @pl.when(moe_active)
    def _moe_wait():
        for cp in moe_copies(g - 1, slot):
            cp.wait()

    @pl.when(g >= 1)
    def _project():
        cur[0].wait()
        xs = xsel_ref[...]

        def up_piece(wbuf, i):
            k0, k1 = KT[i]
            return jnp.dot(xs[:, k0:k1], wbuf[slot, k0:k1, :], preferred_element_type=_F32)

        pieces = [(wgbuf, i) for i in range(len(KT))] + [(wubuf, i) for i in range(len(KT))]
        parts = []
        for c in range(NCH):
            qproj(c)
            parts.append(up_piece(*pieces[c]))
            if c >= NCH - 2:
                parts.append(up_piece(*pieces[c + 2]))
        deferred_oproj(wobuf[(g + 2) % 3], g - 1)
        gate = sum(parts[1:len(KT)], parts[0])
        up = sum(parts[len(KT) + 1:], parts[len(KT)])
        hb_ref[...] = ((gate * jax.nn.sigmoid(gate)) * up).astype(_BF16)

    for cp in cur[1:]:
        cp.wait()

    @pl.when(g + 1 < HKV)
    def _prefetch_attn():
        for cp in attn_copies(g + 1, 1 - slot):
            cp.start()

    @pl.when(g < NF)
    def _prefetch_moe():
        for cp in moe_copies(g, 1 - slot):
            cp.start()


    k = kbuf[slot]
    v = vbuf[slot]

    def qk(c, h):
        return jax.lax.dot_general(q_ref[c, :, h * DH:(h + 1) * DH], k, _NT,
                                   preferred_element_type=_F32)

    def pv(s):
        m = jnp.max(_tree(s, jnp.maximum), axis=-1, keepdims=True)
        p = jnp.exp2(s - m)
        tiles = [p[:, i * 128:(i + 1) * 128] for i in range(S // 128)]
        acc = None
        for g0 in range(0, len(tiles), 4):
            t = (tiles[g0] + tiles[g0 + 1]) + (tiles[g0 + 2] + tiles[g0 + 3])
            acc = t if acc is None else acc + t
            tiles[g0 + 3] = jnp.minimum(tiles[g0 + 3], acc)
        pb = jnp.concatenate(tiles, axis=-1).astype(_BF16)
        return jnp.dot(pb, v, preferred_element_type=_F32), acc

    hb = hb_ref[...]

    def down_piece(i):
        return jax.lax.dot_general(hb[:, i * 128:(i + 1) * 128],
                                   wdbuf[slot, :, i * 128:(i + 1) * 128], _NT,
                                   preferred_element_type=_F32)

    outs = []
    ys = []
    for c in range(NCH):
        sa = qk(c, 0)
        sb = qk(c, 1)
        ra, rb_ = pv(sa), pv(sb)
        if c < FC // 128:
            ys.append(down_piece(c))
        if c < NCH - 1:
            outs.append((normalize(*ra), normalize(*rb_)))
        else:
            for h, r in enumerate((ra, rb_)):
                raw_ref[h, 0] = r[0]
                raw_ref[h, 1] = r[1]
    y_ref[...] += jnp.where(moe_active, sum(ys[1:], ys[0]), 0.0)
    wo_cur = wobuf[g % 3]
    for c in range(NCH - 1):
        oproj(c, *outs[c], wo_cur, g)

    @pl.when(g == HKV - 1)
    def _epilogue():
        y = y_ref[...] * jax.nn.sigmoid(rsel_ref[:, 0:1])
        yt = jnp.concatenate([y, jnp.zeros((128 - CP, D), _F32)], axis=0).T
        yt = yt.astype(_BF16)
        for c in range(NCH):
            cols = pl.ds(c * TQ, TQ)
            if c == NCH - 1:
                deferred_oproj(wobuf[(HKV - 1) % 3], None)
            selc = jnp.concatenate(
                [sel_ref[:, cols], jnp.zeros((128 - CP, TQ), _BF16)], axis=0)
            upd = jnp.dot(yt, selc, preferred_element_type=_F32)
            hb = 0.5 * (xnt_ref[:, cols].astype(_F32) + upd)
            gate = hb + hb * jnp.tanh(hb)
            obuf[:, cols] = (xt_ref[:, cols].astype(_F32)
                             + acc_ref[:, cols] * gate).astype(_BF16)
            out_copy(c).start()
        for c in range(NCH):
            out_copy(c).wait()


@jax.jit
def pallas_recurrent_scan__gqa_block_cached__moe_arch_mod__prompt_kernel(
    A_x: jax.Array,
    A_k_cache: jax.Array,
    A_v_cache: jax.Array,
    A_wq: jax.Array,
    A_wo: jax.Array,
    B_x: jax.Array,
    B_w_r: jax.Array,
    B_w_gate: jax.Array,
    B_w_up: jax.Array,
    B_w_down: jax.Array,
):
    xt = A_x.reshape(S, D).T
    k = A_k_cache.reshape(HKV, S, DH)
    v = A_v_cache.reshape(HKV, S, DH)
    wot = A_wo.T
    wdt = B_w_down.T

    out_t = pl.pallas_call(
        _kernel,
        grid=(HKV,),
        in_specs=[pl.BlockSpec(memory_space=pl.ANY)] * 9,
        out_specs=pl.BlockSpec(memory_space=pl.ANY),
        out_shape=jax.ShapeDtypeStruct((D, S), A_x.dtype),
        scratch_shapes=[
            pltpu.VMEM((D, S), _BF16),
            pltpu.VMEM((D,), _BF16),
            pltpu.VMEM((2, S, DH), _BF16),
            pltpu.VMEM((2, S, DH), _BF16),
            pltpu.VMEM((2, D, GW), _BF16),
            pltpu.VMEM((3, D, GW), _BF16),
            pltpu.VMEM((2, D, FC), _BF16),
            pltpu.VMEM((2, D, FC), _BF16),
            pltpu.VMEM((2, D, FC), _BF16),
            pltpu.VMEM((D, S), _BF16),
            pltpu.VMEM((S, D), _BF16),
            pltpu.VMEM((D, S), _BF16),
            pltpu.VMEM((D, S), _F32),
            pltpu.VMEM((CP, S), _BF16),
            pltpu.VMEM((CP, D), _BF16),
            pltpu.VMEM((CP, 128), _F32),
            pltpu.VMEM((CP, D), _F32),
            pltpu.VMEM((REP, 2, TQ, 128), _F32),
            pltpu.VMEM((NCH, TQ, GW), _BF16),
            pltpu.VMEM((CP, FC), _BF16),
            pltpu.SemaphoreType.DMA((NCH,)),
            pltpu.SemaphoreType.DMA((NCH,)),
            pltpu.SemaphoreType.DMA((1,)),
            pltpu.SemaphoreType.DMA((2, 4)),
            pltpu.SemaphoreType.DMA((2, 3)),
        ],
        compiler_params=pltpu.CompilerParams(
            dimension_semantics=("arbitrary",),
            vmem_limit_bytes=126 * 1024 * 1024,
            disable_bounds_checks=True,
        ),
        name="fused_gqa_mod",
    )(xt, k, v, A_wq, wot, B_w_r, B_w_gate, B_w_up, wdt)
    return out_t.T.reshape(1, S, D)
```

```python
import math

import jax
import jax.numpy as jnp
import jax.experimental.pallas as pl
import jax.experimental.pallas.tpu as pltpu

_BF16 = jnp.bfloat16
_F32 = jnp.float32
_I32 = jnp.int32

S = 2048
D = 576
HQ = 32
HKV = 16
DH = 128
REP = HQ // HKV
GW = REP * DH
F = 4608
C = 8
CP = 16
EPS = 1e-5

TQ = 256
NCH = S // TQ
FC = 384
NF = F // FC
NDEF = 5
NNOW = NCH - NDEF
XDEPTH = 2
XAHEAD = 2
ATT_AT = 4
QSCALE = (DH ** -0.5) * math.log2(math.e)

_NT = (((1,), (1,)), ((), ()))


def _rb(x):
    return x.astype(_BF16).astype(_F32)


def _recip(x):
    r = pl.reciprocal(x, approx=True)
    return r * (2.0 - x * r)


def _tree(a, op):
    tiles = [a[:, i * 128:(i + 1) * 128] for i in range(a.shape[1] // 128)]
    while len(tiles) > 1:
        tiles = [op(tiles[i], tiles[i + 1]) for i in range(0, len(tiles), 2)]
    return tiles[0]


def _kernel(xt_hbm, k_hbm, v_hbm, wq_hbm, wot_hbm, wr_hbm, wg_hbm, wu_hbm, wdt_hbm,
            out_hbm,
            xt_ref, wr_ref, kbuf, vbuf, wqbuf, wobuf, wgbuf, wubuf, wdbuf, obuf,
            xn_ref, xnt_ref, acc_ref, sel_ref, xsel_ref, rsel_ref, y_ref,
            raw_ref, q_ref, hb_ref, x_sem, o_sem, w_sem, a_sem, m_sem):
    g = pl.program_id(0)
    slot = g % 2

    def x_copy(c):
        cols = pl.ds(c * TQ, TQ)
        return pltpu.make_async_copy(xt_hbm.at[:, cols], xt_ref.at[:, cols], x_sem.at[c])

    def out_copy(c):
        cols = pl.ds(c * TQ, TQ)
        return pltpu.make_async_copy(obuf.at[:, cols], out_hbm.at[:, cols], o_sem.at[c])

    def wr_copy():
        return pltpu.make_async_copy(wr_hbm, wr_ref, w_sem.at[0])

    def attn_copies(h, s):
        cols = pl.ds(pl.multiple_of(h * GW, GW), GW)
        return [
            pltpu.make_async_copy(wq_hbm.at[:, cols], wqbuf.at[s], a_sem.at[s, 0]),
            pltpu.make_async_copy(k_hbm.at[h], kbuf.at[s], a_sem.at[s, 1]),
            pltpu.make_async_copy(v_hbm.at[h], vbuf.at[s], a_sem.at[s, 2]),
            pltpu.make_async_copy(wot_hbm.at[:, cols], wobuf.at[h % 3], a_sem.at[s, 3]),
        ]

    def moe_copies(j, s):
        cols = pl.ds(pl.multiple_of(j * FC, 128), FC)
        return [
            pltpu.make_async_copy(wg_hbm.at[:, cols], wgbuf.at[s], m_sem.at[s, 0]),
            pltpu.make_async_copy(wu_hbm.at[:, cols], wubuf.at[s], m_sem.at[s, 1]),
            pltpu.make_async_copy(wdt_hbm.at[:, cols], wdbuf.at[s], m_sem.at[s, 2]),
        ]

    def qproj(c):
        q = jnp.dot(xn_ref[pl.ds(c * TQ, TQ), :], wqbuf[slot], preferred_element_type=_F32)
        q_ref[c] = (q * QSCALE).astype(_BF16)

    def normalize(o, part):
        l = jnp.sum(part, axis=-1, keepdims=True)
        return (o * _recip(l)).astype(_BF16)

    def oproj(c, oa, ob, wo, nheads_done):
        o2 = jnp.concatenate([oa, ob], axis=-1)
        prev = acc_ref[:, pl.ds(c * TQ, TQ)]
        if nheads_done is not None:
            prev = jnp.where(nheads_done > 0, prev, 0.0)
        return prev + jax.lax.dot_general(wo, o2, _NT, preferred_element_type=_F32)

    def deferred_oproj(i, wo, nheads_done):
        oa = normalize(raw_ref[i, 0, 0], raw_ref[i, 0, 1])
        ob = normalize(raw_ref[i, 1, 0], raw_ref[i, 1, 1])
        return oproj(NNOW + i, oa, ob, wo, nheads_done)

    @pl.when(g == 0)
    def _prologue():
        first = attn_copies(0, 0)
        wr_copy().start()
        for c in range(XDEPTH):
            x_copy(c).start()
        first[0].start()
        wr_copy().wait()
        wr = jnp.broadcast_to(wr_ref[...].reshape(1, D), (8, D))

        def layernorm(c):
            cols = pl.ds(c * TQ, TQ)
            x0 = xt_ref[0:16, cols].astype(_F32)[0:1, :]
            s1 = s2 = None
            for r0 in range(0, D, 16):
                d = xt_ref[r0:r0 + 16, cols].astype(_F32) - x0
                s1 = d if s1 is None else s1 + d
                s2 = d * d if s2 is None else s2 + d * d
            md = jnp.sum(s1, axis=0, keepdims=True) * (1.0 / D)
            var = jnp.sum(s2, axis=0, keepdims=True) * (1.0 / D) - md * md
            var = jnp.maximum(var, 0.0)
            mean = _rb(x0 + md)
            inv = _recip(_rb(jnp.sqrt(_rb(_rb(var) + EPS))))
            xn32 = jnp.concatenate(
                [_rb(xt_ref[r0:r0 + 64, cols].astype(_F32) - mean) * inv
                 for r0 in range(0, D, 64)], axis=0)
            xn = xn32.astype(_BF16)
            xnt_ref[:, cols] = xn
            xn_ref[cols, :] = xn32.T.astype(_BF16)
            return jnp.dot(wr, xn, preferred_element_type=_F32)[0:1, :]

        rs = []
        for c in range(0, NCH, 2):
            x_copy(c).wait()
            x_copy(c + 1).wait()
            for cn in (c + XAHEAD, c + XAHEAD + 1):
                if cn < NCH:
                    x_copy(cn).start()
            if c == ATT_AT:
                for cp in first[1:]:
                    cp.start()
            if c == 2:
                first[0].wait()
            if c >= 2:
                qproj(c - 2)
                qproj(c - 1)
            rs.append(layernorm(c))
            rs.append(layernorm(c + 1))
        qproj(NCH - 2)
        qproj(NCH - 1)
        r = _rb(jnp.concatenate(rs, axis=1)) + 0.0
        pos = jax.lax.broadcasted_iota(_I32, (1, S), 1)
        bits = pltpu.bitcast(r, _I32)
        key = jnp.where(bits < 0, bits ^ 0x7FFF0000, bits) | (S - 1 - pos)
        row16 = jax.lax.broadcasted_iota(_I32, (16, D), 0)
        sels, rsel, xsel = [], [], []
        for c in range(C):
            m = jnp.max(key, axis=1, keepdims=True)
            hit = key == m
            sels.append(hit.astype(_F32))
            hi = jnp.broadcast_to(m, (1, 128)) & jnp.int32(-65536)
            rsel.append(pltpu.bitcast(jnp.where(hi < 0, hi ^ 0x7FFF0000, hi), _F32))
            key = jnp.where(hit, jnp.iinfo(jnp.int32).min, key)
            idx = (S - 1) - (m[0, 0] & (S - 1))
            blk = xn_ref[pl.ds(pl.multiple_of((idx // 16) * 16, 16), 16), :].astype(_F32)
            xsel.append(jnp.sum(jnp.where(row16 == idx % 16, blk, 0.0), axis=0, keepdims=True))
        sel_ref[...] = jnp.concatenate(
            sels + [jnp.zeros((CP - C, S), _F32)], axis=0).astype(_BF16)
        rsel_ref[...] = jnp.concatenate(rsel + [jnp.zeros((CP - C, 128), _F32)], axis=0)
        xsel_ref[...] = jnp.concatenate(
            xsel + [jnp.zeros((CP - C, D), _F32)], axis=0).astype(_BF16)
        y_ref[...] = jnp.zeros_like(y_ref)
        hb_ref[...] = jnp.zeros_like(hb_ref)

    moe_active = jnp.logical_and(g >= 1, g <= NF)
    cur = attn_copies(g, slot)
    KT = [(k0, min(k0 + 128, D)) for k0 in range(0, D, 128)]

    @pl.when(moe_active)
    def _moe_wait():
        for cp in moe_copies(g - 1, slot):
            cp.wait()

    @pl.when(g >= 1)
    def _project():
        cur[0].wait()
        xs = xsel_ref[...]

        def up_piece(wbuf, i):
            k0, k1 = KT[i]
            return jnp.dot(xs[:, k0:k1], wbuf[slot, k0:k1, :], preferred_element_type=_F32)

        pieces = [(wgbuf, i) for i in range(len(KT))] + [(wubuf, i) for i in range(len(KT))]
        parts = []
        wo_prev = wobuf[(g + 2) % 3]
        for c in range(NCH):
            qproj(c)
            parts.append(up_piece(*pieces[c]))
            if c >= NCH - 2:
                parts.append(up_piece(*pieces[c + 2]))
            i = c - (NCH - NDEF)
            if i >= 0:
                acc_ref[:, pl.ds((NNOW + i) * TQ, TQ)] = deferred_oproj(i, wo_prev, g - 1)
        gate = sum(parts[1:len(KT)], parts[0])
        up = sum(parts[len(KT) + 1:], parts[len(KT)])
        hb_ref[...] = ((gate * jax.nn.sigmoid(gate)) * up).astype(_BF16)

    for cp in cur[1:]:
        cp.wait()

    @pl.when(g + 1 < HKV)
    def _prefetch_attn():
        for cp in attn_copies(g + 1, 1 - slot):
            cp.start()

    @pl.when(g < NF)
    def _prefetch_moe():
        for cp in moe_copies(g, 1 - slot):
            cp.start()

    k = kbuf[slot]
    v = vbuf[slot]

    def qk(c, h):
        return jax.lax.dot_general(q_ref[c, :, h * DH:(h + 1) * DH], k, _NT,
                                   preferred_element_type=_F32)

    def pv(s):
        m = jnp.max(_tree(s, jnp.maximum), axis=-1, keepdims=True)
        p = jnp.exp2(s - m)
        tiles = [p[:, i * 128:(i + 1) * 128] for i in range(S // 128)]
        acc = None
        for g0 in range(0, len(tiles), 4):
            t = (tiles[g0] + tiles[g0 + 1]) + (tiles[g0 + 2] + tiles[g0 + 3])
            acc = t if acc is None else acc + t
            tiles[g0 + 3] = jnp.minimum(tiles[g0 + 3], acc)
        pb = jnp.concatenate(tiles, axis=-1).astype(_BF16)
        return jnp.dot(pb, v, preferred_element_type=_F32), acc

    hb = hb_ref[...]

    def down_piece(i):
        return jax.lax.dot_general(hb[:, i * 128:(i + 1) * 128],
                                   wdbuf[slot, :, i * 128:(i + 1) * 128], _NT,
                                   preferred_element_type=_F32)

    outs = []
    ys = []
    for c in range(NCH):
        sa = qk(c, 0)
        sb = qk(c, 1)
        ra, rb_ = pv(sa), pv(sb)
        if c < FC // 128:
            ys.append(down_piece(c))
        if c < NNOW:
            outs.append((normalize(*ra), normalize(*rb_)))
        else:
            for h, r in enumerate((ra, rb_)):
                raw_ref[c - NNOW, h, 0] = r[0]
                raw_ref[c - NNOW, h, 1] = r[1]
    y_ref[...] += jnp.where(moe_active, sum(ys[1:], ys[0]), 0.0)
    wo_cur = wobuf[g % 3]
    for c in range(NNOW):
        acc_ref[:, pl.ds(c * TQ, TQ)] = oproj(c, *outs[c], wo_cur, g)

    @pl.when(g == HKV - 1)
    def _epilogue():
        y = y_ref[...] * jax.nn.sigmoid(rsel_ref[:, 0:1])
        yt = jnp.concatenate([y, jnp.zeros((128 - CP, D), _F32)], axis=0).T
        yt = yt.astype(_BF16)
        wo_last = wobuf[(HKV - 1) % 3]
        upds, late = [], []
        for c in range(NCH):
            if c >= NNOW:
                late.append(deferred_oproj(c - NNOW, wo_last, None))
            selc = jnp.concatenate(
                [sel_ref[:, pl.ds(c * TQ, TQ)], jnp.zeros((128 - CP, TQ), _BF16)], axis=0)
            upds.append(jnp.dot(yt, selc, preferred_element_type=_F32))
        for c in range(NCH):
            cols = pl.ds(c * TQ, TQ)
            attn = acc_ref[:, cols] if c < NNOW else late[c - NNOW]
            hb = 0.5 * (xnt_ref[:, cols].astype(_F32) + upds[c])
            gate = hb + hb * jnp.tanh(hb)
            obuf[:, cols] = (xt_ref[:, cols].astype(_F32) + attn * gate).astype(_BF16)
            out_copy(c).start()
        for c in range(NCH):
            out_copy(c).wait()


@jax.jit
def pallas_recurrent_scan__gqa_block_cached__moe_arch_mod__prompt_kernel(
    A_x: jax.Array,
    A_k_cache: jax.Array,
    A_v_cache: jax.Array,
    A_wq: jax.Array,
    A_wo: jax.Array,
    B_x: jax.Array,
    B_w_r: jax.Array,
    B_w_gate: jax.Array,
    B_w_up: jax.Array,
    B_w_down: jax.Array,
):
    xt = A_x.reshape(S, D).T
    k = A_k_cache.reshape(HKV, S, DH)
    v = A_v_cache.reshape(HKV, S, DH)
    wot = A_wo.T
    wdt = B_w_down.T

    out_t = pl.pallas_call(
        _kernel,
        grid=(HKV,),
        in_specs=[pl.BlockSpec(memory_space=pl.ANY)] * 9,
        out_specs=pl.BlockSpec(memory_space=pl.ANY),
        out_shape=jax.ShapeDtypeStruct((D, S), A_x.dtype),
        scratch_shapes=[
            pltpu.VMEM((D, S), _BF16),
            pltpu.VMEM((D,), _BF16),
            pltpu.VMEM((2, S, DH), _BF16),
            pltpu.VMEM((2, S, DH), _BF16),
            pltpu.VMEM((2, D, GW), _BF16),
            pltpu.VMEM((3, D, GW), _BF16),
            pltpu.VMEM((2, D, FC), _BF16),
            pltpu.VMEM((2, D, FC), _BF16),
            pltpu.VMEM((2, D, FC), _BF16),
            pltpu.VMEM((D, S), _BF16),
            pltpu.VMEM((S, D), _BF16),
            pltpu.VMEM((D, S), _BF16),
            pltpu.VMEM((D, S), _F32),
            pltpu.VMEM((CP, S), _BF16),
            pltpu.VMEM((CP, D), _BF16),
            pltpu.VMEM((CP, 128), _F32),
            pltpu.VMEM((CP, D), _F32),
            pltpu.VMEM((NDEF, REP, 2, TQ, 128), _F32),
            pltpu.VMEM((NCH, TQ, GW), _BF16),
            pltpu.VMEM((CP, FC), _BF16),
            pltpu.SemaphoreType.DMA((NCH,)),
            pltpu.SemaphoreType.DMA((NCH,)),
            pltpu.SemaphoreType.DMA((1,)),
            pltpu.SemaphoreType.DMA((2, 4)),
            pltpu.SemaphoreType.DMA((2, 3)),
        ],
        compiler_params=pltpu.CompilerParams(
            dimension_semantics=("arbitrary",),
            vmem_limit_bytes=126 * 1024 * 1024,
            disable_bounds_checks=True,
        ),
        name="fused_gqa_mod",
    )(xt, k, v, A_wq, wot, B_w_r, B_w_gate, B_w_up, wdt)
    return out_t.T.reshape(1, S, D)
```

```python
import math

import jax
import jax.numpy as jnp
import jax.experimental.pallas as pl
import jax.experimental.pallas.tpu as pltpu

_BF16 = jnp.bfloat16
_F32 = jnp.float32
_I32 = jnp.int32

S = 2048
D = 576
HQ = 32
HKV = 16
DH = 128
REP = HQ // HKV
GW = REP * DH
F = 4608
C = 8
CP = 16
EPS = 1e-5

TQ = 256
NCH = S // TQ
FC = 384
NF = F // FC
NDEF = 5
NNOW = NCH - NDEF
XDEPTH = 2
XAHEAD = 2
ATT_AT = 4
QSCALE = (DH ** -0.5) * math.log2(math.e)

_NT = (((1,), (1,)), ((), ()))


def _rb(x):
    return x.astype(_BF16).astype(_F32)


def _recip(x):
    r = pl.reciprocal(x, approx=True)
    return r * (2.0 - x * r)


def _tree(a, op):
    tiles = [a[:, i * 128:(i + 1) * 128] for i in range(a.shape[1] // 128)]
    while len(tiles) > 1:
        tiles = [op(tiles[i], tiles[i + 1]) for i in range(0, len(tiles), 2)]
    return tiles[0]


def _kernel(xt_hbm, k_hbm, v_hbm, wq_hbm, wot_hbm, wr_hbm, wg_hbm, wu_hbm, wdt_hbm,
            out_hbm,
            xt_ref, wr_ref, kbuf, vbuf, wqbuf, wobuf, wgbuf, wubuf, wdbuf, obuf,
            xn_ref, xnt_ref, acc_ref, sel_ref, xsel_ref, rsel_ref, y_ref,
            raw_ref, q_ref, hb_ref, x_sem, o_sem, w_sem, a_sem, m_sem):
    g = pl.program_id(0)
    slot = g % 2

    def x_copy(c):
        cols = pl.ds(c * TQ, TQ)
        return pltpu.make_async_copy(xt_hbm.at[:, cols], xt_ref.at[:, cols], x_sem.at[c])

    def out_copy(c):
        cols = pl.ds(c * TQ, TQ)
        return pltpu.make_async_copy(obuf.at[:, cols], out_hbm.at[:, cols], o_sem.at[c])

    def wr_copy():
        return pltpu.make_async_copy(wr_hbm, wr_ref, w_sem.at[0])

    def attn_copies(h, s):
        cols = pl.ds(pl.multiple_of(h * GW, GW), GW)
        return [
            pltpu.make_async_copy(wq_hbm.at[:, cols], wqbuf.at[s], a_sem.at[s, 0]),
            pltpu.make_async_copy(k_hbm.at[h], kbuf.at[s], a_sem.at[s, 1]),
            pltpu.make_async_copy(v_hbm.at[h], vbuf.at[s], a_sem.at[s, 2]),
            pltpu.make_async_copy(wot_hbm.at[:, cols], wobuf.at[h % 4], a_sem.at[s, 3]),
        ]

    def moe_copies(j, s):
        cols = pl.ds(pl.multiple_of(j * FC, 128), FC)
        return [
            pltpu.make_async_copy(wg_hbm.at[:, cols], wgbuf.at[s], m_sem.at[s, 0]),
            pltpu.make_async_copy(wu_hbm.at[:, cols], wubuf.at[s], m_sem.at[s, 1]),
            pltpu.make_async_copy(wdt_hbm.at[:, cols], wdbuf.at[s], m_sem.at[s, 2]),
        ]

    def qproj(c):
        q = jnp.dot(xn_ref[pl.ds(c * TQ, TQ), :], wqbuf[slot], preferred_element_type=_F32)
        q_ref[c] = (q * QSCALE).astype(_BF16)

    def normalize(o, part):
        l = jnp.sum(part, axis=-1, keepdims=True)
        return (o * _recip(l)).astype(_BF16)

    def oproj(c, oa, ob, wo, nheads_done):
        o2 = jnp.concatenate([oa, ob], axis=-1)
        prev = acc_ref[:, pl.ds(c * TQ, TQ)]
        if nheads_done is not None:
            prev = jnp.where(nheads_done > 0, prev, 0.0)
        return prev + jax.lax.dot_general(wo, o2, _NT, preferred_element_type=_F32)

    def deferred_oproj(i, wo, nheads_done):
        oa = normalize(raw_ref[i, 0, 0], raw_ref[i, 0, 1])
        ob = normalize(raw_ref[i, 1, 0], raw_ref[i, 1, 1])
        return oproj(NNOW + i, oa, ob, wo, nheads_done)

    @pl.when(g == 0)
    def _prologue():
        first = attn_copies(0, 0)
        wr_copy().start()
        for c in range(XDEPTH):
            x_copy(c).start()
        first[0].start()
        wr_copy().wait()
        wr = jnp.broadcast_to(wr_ref[...].reshape(1, D), (8, D))

        def layernorm(c):
            cols = pl.ds(c * TQ, TQ)
            x0 = xt_ref[0:16, cols].astype(_F32)[0:1, :]
            s1 = s2 = None
            for r0 in range(0, D, 16):
                d = xt_ref[r0:r0 + 16, cols].astype(_F32) - x0
                s1 = d if s1 is None else s1 + d
                s2 = d * d if s2 is None else s2 + d * d
            md = jnp.sum(s1, axis=0, keepdims=True) * (1.0 / D)
            var = jnp.sum(s2, axis=0, keepdims=True) * (1.0 / D) - md * md
            var = jnp.maximum(var, 0.0)
            mean = _rb(x0 + md)
            inv = _recip(_rb(jnp.sqrt(_rb(_rb(var) + EPS))))
            xn32 = jnp.concatenate(
                [_rb(xt_ref[r0:r0 + 64, cols].astype(_F32) - mean) * inv
                 for r0 in range(0, D, 64)], axis=0)
            xn = xn32.astype(_BF16)
            xnt_ref[:, cols] = xn
            xn_ref[cols, :] = xn32.T.astype(_BF16)
            return jnp.dot(wr, xn, preferred_element_type=_F32)[0:1, :]

        rs = []
        for c in range(0, NCH, 2):
            x_copy(c).wait()
            x_copy(c + 1).wait()
            for cn in (c + XAHEAD, c + XAHEAD + 1):
                if cn < NCH:
                    x_copy(cn).start()
            if c == ATT_AT:
                for cp in first[1:]:
                    cp.start()
            if c == 2:
                first[0].wait()
            if c >= 2:
                qproj(c - 2)
                qproj(c - 1)
            rs.append(layernorm(c))
            rs.append(layernorm(c + 1))
        qproj(NCH - 2)
        qproj(NCH - 1)
        r = _rb(jnp.concatenate(rs, axis=1)) + 0.0
        pos = jax.lax.broadcasted_iota(_I32, (1, S), 1)
        bits = pltpu.bitcast(r, _I32)
        key = jnp.where(bits < 0, bits ^ 0x7FFF0000, bits) | (S - 1 - pos)
        row16 = jax.lax.broadcasted_iota(_I32, (16, D), 0)
        sels, rsel, xsel = [], [], []
        for c in range(C):
            m = jnp.max(key, axis=1, keepdims=True)
            hit = key == m
            sels.append(hit.astype(_F32))
            hi = jnp.broadcast_to(m, (1, 128)) & jnp.int32(-65536)
            rsel.append(pltpu.bitcast(jnp.where(hi < 0, hi ^ 0x7FFF0000, hi), _F32))
            key = jnp.where(hit, jnp.iinfo(jnp.int32).min, key)
            idx = (S - 1) - (m[0, 0] & (S - 1))
            blk = xn_ref[pl.ds(pl.multiple_of((idx // 16) * 16, 16), 16), :].astype(_F32)
            xsel.append(jnp.sum(jnp.where(row16 == idx % 16, blk, 0.0), axis=0, keepdims=True))
        sel_ref[...] = jnp.concatenate(
            sels + [jnp.zeros((CP - C, S), _F32)], axis=0).astype(_BF16)
        rsel_ref[...] = jnp.concatenate(rsel + [jnp.zeros((CP - C, 128), _F32)], axis=0)
        xsel_ref[...] = jnp.concatenate(
            xsel + [jnp.zeros((CP - C, D), _F32)], axis=0).astype(_BF16)
        y_ref[...] = jnp.zeros_like(y_ref)
        hb_ref[...] = jnp.zeros_like(hb_ref)

    moe_active = jnp.logical_and(g >= 1, g <= NF)
    cur = attn_copies(g, slot)
    KT = [(k0, min(k0 + 128, D)) for k0 in range(0, D, 128)]

    @pl.when(moe_active)
    def _moe_wait():
        for cp in moe_copies(g - 1, slot):
            cp.wait()

    @pl.when(g >= 1)
    def _project():
        cur[0].wait()
        xs = xsel_ref[...]

        def up_piece(wbuf, i):
            k0, k1 = KT[i]
            return jnp.dot(xs[:, k0:k1], wbuf[slot, k0:k1, :], preferred_element_type=_F32)

        pieces = [(wgbuf, i) for i in range(len(KT))] + [(wubuf, i) for i in range(len(KT))]
        parts = []
        wo_prev = wobuf[(g + 3) % 4]
        for c in range(NCH):
            qproj(c)
            parts.append(up_piece(*pieces[len(parts)]))
            if c < len(pieces) - NCH:
                parts.append(up_piece(*pieces[len(parts)]))
            i = c - (NCH - NDEF)
            if i >= 0:
                acc_ref[:, pl.ds((NNOW + i) * TQ, TQ)] = deferred_oproj(i, wo_prev, g - 1)
        gate = sum(parts[1:len(KT)], parts[0])
        up = sum(parts[len(KT) + 1:], parts[len(KT)])
        hb_ref[...] = ((gate * jax.nn.sigmoid(gate)) * up).astype(_BF16)

    for cp in cur[1:]:
        cp.wait()

    k = kbuf[slot]
    v = vbuf[slot]

    def qk(c, h):
        return jax.lax.dot_general(q_ref[c, :, h * DH:(h + 1) * DH], k, _NT,
                                   preferred_element_type=_F32)

    def pv(s):
        m = jnp.max(_tree(s, jnp.maximum), axis=-1, keepdims=True)
        p = jnp.exp2(s - m)
        tiles = [p[:, i * 128:(i + 1) * 128] for i in range(S // 128)]
        acc = None
        for g0 in range(0, len(tiles), 4):
            t = (tiles[g0] + tiles[g0 + 1]) + (tiles[g0 + 2] + tiles[g0 + 3])
            acc = t if acc is None else acc + t
            tiles[g0 + 3] = jnp.minimum(tiles[g0 + 3], acc)
        pb = jnp.concatenate(tiles, axis=-1).astype(_BF16)
        return jnp.dot(pb, v, preferred_element_type=_F32), acc

    hb = hb_ref[...]

    def down_piece(i):
        return jax.lax.dot_general(hb[:, i * 128:(i + 1) * 128],
                                   wdbuf[slot, :, i * 128:(i + 1) * 128], _NT,
                                   preferred_element_type=_F32)

    def prefetch():
        @pl.when(g + 1 < HKV)
        def _prefetch_attn():
            for cp in attn_copies(g + 1, 1 - slot):
                cp.start()

        @pl.when(g < NF)
        def _prefetch_moe():
            for cp in moe_copies(g, 1 - slot):
                cp.start()

    outs = []
    ys = []
    for c in range(NCH):
        sa = qk(c, 0)
        sb = qk(c, 1)
        ra, rb_ = pv(sa), pv(sb)
        if c == 0:
            prefetch()
        if c < FC // 128:
            ys.append(down_piece(c))
        if c < NNOW:
            outs.append((normalize(*ra), normalize(*rb_)))
        else:
            for h, r in enumerate((ra, rb_)):
                raw_ref[c - NNOW, h, 0] = r[0]
                raw_ref[c - NNOW, h, 1] = r[1]
    y_ref[...] += jnp.where(moe_active, sum(ys[1:], ys[0]), 0.0)
    wo_cur = wobuf[g % 4]
    for c in range(NNOW):
        acc_ref[:, pl.ds(c * TQ, TQ)] = oproj(c, *outs[c], wo_cur, g)

    @pl.when(g == HKV - 1)
    def _epilogue():
        y = y_ref[...] * jax.nn.sigmoid(rsel_ref[:, 0:1])
        yt = jnp.concatenate([y, jnp.zeros((128 - CP, D), _F32)], axis=0).T
        yt = yt.astype(_BF16)
        wo_last = wobuf[(HKV - 1) % 4]
        upds, late = [], []
        for c in range(NCH):
            if c >= NNOW:
                late.append(deferred_oproj(c - NNOW, wo_last, None))
            selc = jnp.concatenate(
                [sel_ref[:, pl.ds(c * TQ, TQ)], jnp.zeros((128 - CP, TQ), _BF16)], axis=0)
            upds.append(jnp.dot(yt, selc, preferred_element_type=_F32))
        for c in range(NCH):
            cols = pl.ds(c * TQ, TQ)
            attn = acc_ref[:, cols] if c < NNOW else late[c - NNOW]
            hb = 0.5 * (xnt_ref[:, cols].astype(_F32) + upds[c])
            gate = hb + hb * jnp.tanh(hb)
            obuf[:, cols] = (xt_ref[:, cols].astype(_F32) + attn * gate).astype(_BF16)
            out_copy(c).start()
        for c in range(NCH):
            out_copy(c).wait()


@jax.jit
def pallas_recurrent_scan__gqa_block_cached__moe_arch_mod__prompt_kernel(
    A_x: jax.Array,
    A_k_cache: jax.Array,
    A_v_cache: jax.Array,
    A_wq: jax.Array,
    A_wo: jax.Array,
    B_x: jax.Array,
    B_w_r: jax.Array,
    B_w_gate: jax.Array,
    B_w_up: jax.Array,
    B_w_down: jax.Array,
):
    xt = A_x.reshape(S, D).T
    k = A_k_cache.reshape(HKV, S, DH)
    v = A_v_cache.reshape(HKV, S, DH)
    wot = A_wo.T
    wdt = B_w_down.T

    out_t = pl.pallas_call(
        _kernel,
        grid=(HKV,),
        in_specs=[pl.BlockSpec(memory_space=pl.ANY)] * 9,
        out_specs=pl.BlockSpec(memory_space=pl.ANY),
        out_shape=jax.ShapeDtypeStruct((D, S), A_x.dtype),
        scratch_shapes=[
            pltpu.VMEM((D, S), _BF16),
            pltpu.VMEM((D,), _BF16),
            pltpu.VMEM((2, S, DH), _BF16),
            pltpu.VMEM((2, S, DH), _BF16),
            pltpu.VMEM((2, D, GW), _BF16),
            pltpu.VMEM((4, D, GW), _BF16),
            pltpu.VMEM((2, D, FC), _BF16),
            pltpu.VMEM((2, D, FC), _BF16),
            pltpu.VMEM((2, D, FC), _BF16),
            pltpu.VMEM((D, S), _BF16),
            pltpu.VMEM((S, D), _BF16),
            pltpu.VMEM((D, S), _BF16),
            pltpu.VMEM((D, S), _F32),
            pltpu.VMEM((CP, S), _BF16),
            pltpu.VMEM((CP, D), _BF16),
            pltpu.VMEM((CP, 128), _F32),
            pltpu.VMEM((CP, D), _F32),
            pltpu.VMEM((NDEF, REP, 2, TQ, 128), _F32),
            pltpu.VMEM((NCH, TQ, GW), _BF16),
            pltpu.VMEM((CP, FC), _BF16),
            pltpu.SemaphoreType.DMA((NCH,)),
            pltpu.SemaphoreType.DMA((NCH,)),
            pltpu.SemaphoreType.DMA((1,)),
            pltpu.SemaphoreType.DMA((2, 4)),
            pltpu.SemaphoreType.DMA((2, 3)),
        ],
        compiler_params=pltpu.CompilerParams(
            dimension_semantics=("arbitrary",),
            vmem_limit_bytes=126 * 1024 * 1024,
            disable_bounds_checks=True,
        ),
        name="fused_gqa_mod",
    )(xt, k, v, A_wq, wot, B_w_r, B_w_gate, B_w_up, wdt)
    return out_t.T.reshape(1, S, D)
```

```python
import math

import jax
import jax.numpy as jnp
import jax.experimental.pallas as pl
import jax.experimental.pallas.tpu as pltpu

_BF16 = jnp.bfloat16
_F32 = jnp.float32
_I32 = jnp.int32

S = 2048
D = 576
HQ = 32
HKV = 16
DH = 128
REP = HQ // HKV
GW = REP * DH
F = 4608
C = 8
CP = 16
EPS = 1e-5

TQ = 256
NCH = S // TQ
FC = 384
NF = F // FC
NDEF = 5
NNOW = NCH - NDEF
XDEPTH = 2
XAHEAD = 2
ATT_AT = 4
QSCALE = (DH ** -0.5) * math.log2(math.e)

_NT = (((1,), (1,)), ((), ()))


def _rb(x):
    return x.astype(_BF16).astype(_F32)


def _recip(x):
    r = pl.reciprocal(x, approx=True)
    return r * (2.0 - x * r)


def _tree(a, op):
    tiles = [a[:, i * 128:(i + 1) * 128] for i in range(a.shape[1] // 128)]
    while len(tiles) > 1:
        tiles = [op(tiles[i], tiles[i + 1]) for i in range(0, len(tiles), 2)]
    return tiles[0]


def _kernel(xt_hbm, k_hbm, v_hbm, wq_hbm, wot_hbm, wr_hbm, wg_hbm, wu_hbm, wdt_hbm,
            out_hbm,
            xt_ref, wr_ref, kbuf, vbuf, wqbuf, wobuf, wgbuf, wubuf, wdbuf, obuf,
            xn_ref, xnt_ref, acc_ref, sel_ref, xsel_ref, rsel_ref, y_ref,
            raw_ref, q_ref, hb_ref, yt_ref, x_sem, o_sem, w_sem, a_sem, m_sem):
    g = pl.program_id(0)
    slot = g % 2

    def x_copy(c):
        cols = pl.ds(c * TQ, TQ)
        return pltpu.make_async_copy(xt_hbm.at[:, cols], xt_ref.at[:, cols], x_sem.at[c])

    def out_copy(c):
        cols = pl.ds(c * TQ, TQ)
        return pltpu.make_async_copy(obuf.at[:, cols], out_hbm.at[:, cols], o_sem.at[c])

    def wr_copy():
        return pltpu.make_async_copy(wr_hbm, wr_ref, w_sem.at[0])

    def attn_copies(h, s):
        cols = pl.ds(pl.multiple_of(h * GW, GW), GW)
        return [
            pltpu.make_async_copy(wq_hbm.at[:, cols], wqbuf.at[s], a_sem.at[s, 0]),
            pltpu.make_async_copy(k_hbm.at[h], kbuf.at[s], a_sem.at[s, 1]),
            pltpu.make_async_copy(v_hbm.at[h], vbuf.at[s], a_sem.at[s, 2]),
            pltpu.make_async_copy(wot_hbm.at[:, cols], wobuf.at[h % 4], a_sem.at[s, 3]),
        ]

    def moe_copies(j, s):
        cols = pl.ds(pl.multiple_of(j * FC, 128), FC)
        return [
            pltpu.make_async_copy(wg_hbm.at[:, cols], wgbuf.at[s], m_sem.at[s, 0]),
            pltpu.make_async_copy(wu_hbm.at[:, cols], wubuf.at[s], m_sem.at[s, 1]),
            pltpu.make_async_copy(wdt_hbm.at[:, cols], wdbuf.at[s], m_sem.at[s, 2]),
        ]

    def qproj(c):
        q = jnp.dot(xn_ref[pl.ds(c * TQ, TQ), :], wqbuf[slot], preferred_element_type=_F32)
        q_ref[c] = (q * QSCALE).astype(_BF16)

    def normalize(o, part):
        l = jnp.sum(part, axis=-1, keepdims=True)
        return (o * _recip(l)).astype(_BF16)

    def oproj(c, oa, ob, wo, nheads_done):
        o2 = jnp.concatenate([oa, ob], axis=-1)
        prev = acc_ref[:, pl.ds(c * TQ, TQ)]
        if nheads_done is not None:
            prev = jnp.where(nheads_done > 0, prev, 0.0)
        return prev + jax.lax.dot_general(wo, o2, _NT, preferred_element_type=_F32)

    def deferred_oproj(i, wo, nheads_done):
        oa = normalize(raw_ref[i, 0, 0], raw_ref[i, 0, 1])
        ob = normalize(raw_ref[i, 1, 0], raw_ref[i, 1, 1])
        return oproj(NNOW + i, oa, ob, wo, nheads_done)

    @pl.when(g == 0)
    def _prologue():
        first = attn_copies(0, 0)
        wr_copy().start()
        for c in range(XDEPTH):
            x_copy(c).start()
        first[0].start()
        wr_copy().wait()
        wr = jnp.broadcast_to(wr_ref[...].reshape(1, D), (8, D))

        def layernorm(c):
            cols = pl.ds(c * TQ, TQ)
            x0 = xt_ref[0:16, cols].astype(_F32)[0:1, :]
            s1 = s2 = None
            for r0 in range(0, D, 16):
                d = xt_ref[r0:r0 + 16, cols].astype(_F32) - x0
                s1 = d if s1 is None else s1 + d
                s2 = d * d if s2 is None else s2 + d * d
            md = jnp.sum(s1, axis=0, keepdims=True) * (1.0 / D)
            var = jnp.sum(s2, axis=0, keepdims=True) * (1.0 / D) - md * md
            var = jnp.maximum(var, 0.0)
            mean = _rb(x0 + md)
            inv = _recip(_rb(jnp.sqrt(_rb(_rb(var) + EPS))))
            xn32 = jnp.concatenate(
                [_rb(xt_ref[r0:r0 + 64, cols].astype(_F32) - mean) * inv
                 for r0 in range(0, D, 64)], axis=0)
            xn = xn32.astype(_BF16)
            xnt_ref[:, cols] = xn
            xn_ref[cols, :] = xn32.T.astype(_BF16)
            return jnp.dot(wr, xn, preferred_element_type=_F32)[0:1, :]

        rs = []
        for c in range(0, NCH, 2):
            x_copy(c).wait()
            x_copy(c + 1).wait()
            for cn in (c + XAHEAD, c + XAHEAD + 1):
                if cn < NCH:
                    x_copy(cn).start()
            if c == ATT_AT:
                for cp in first[1:]:
                    cp.start()
            if c == 2:
                first[0].wait()
            if c >= 2:
                qproj(c - 2)
                qproj(c - 1)
            rs.append(layernorm(c))
            rs.append(layernorm(c + 1))
        qproj(NCH - 2)
        qproj(NCH - 1)
        r = _rb(jnp.concatenate(rs, axis=1)) + 0.0
        pos = jax.lax.broadcasted_iota(_I32, (1, S), 1)
        bits = pltpu.bitcast(r, _I32)
        key = jnp.where(bits < 0, bits ^ 0x7FFF0000, bits) | (S - 1 - pos)
        row16 = jax.lax.broadcasted_iota(_I32, (16, D), 0)
        sels, rsel, xsel = [], [], []
        for c in range(C):
            m = jnp.max(key, axis=1, keepdims=True)
            hit = key == m
            sels.append(hit.astype(_F32))
            hi = jnp.broadcast_to(m, (1, 128)) & jnp.int32(-65536)
            rsel.append(pltpu.bitcast(jnp.where(hi < 0, hi ^ 0x7FFF0000, hi), _F32))
            key = jnp.where(hit, jnp.iinfo(jnp.int32).min, key)
            idx = (S - 1) - (m[0, 0] & (S - 1))
            blk = xn_ref[pl.ds(pl.multiple_of((idx // 16) * 16, 16), 16), :].astype(_F32)
            xsel.append(jnp.sum(jnp.where(row16 == idx % 16, blk, 0.0), axis=0, keepdims=True))
        sel_ref[...] = jnp.concatenate(
            sels + [jnp.zeros((CP - C, S), _F32)], axis=0).astype(_BF16)
        rsel_ref[...] = jnp.concatenate(rsel + [jnp.zeros((CP - C, 128), _F32)], axis=0)
        xsel_ref[...] = jnp.concatenate(
            xsel + [jnp.zeros((CP - C, D), _F32)], axis=0).astype(_BF16)
        y_ref[...] = jnp.zeros_like(y_ref)
        hb_ref[...] = jnp.zeros_like(hb_ref)

    moe_active = jnp.logical_and(g >= 1, g <= NF)
    cur = attn_copies(g, slot)
    KT = [(k0, min(k0 + 128, D)) for k0 in range(0, D, 128)]

    @pl.when(moe_active)
    def _moe_wait():
        for cp in moe_copies(g - 1, slot):
            cp.wait()

    @pl.when(g >= 1)
    def _project():
        cur[0].wait()
        xs = xsel_ref[...]

        def up_piece(wbuf, i):
            k0, k1 = KT[i]
            return jnp.dot(xs[:, k0:k1], wbuf[slot, k0:k1, :], preferred_element_type=_F32)

        pieces = [(wgbuf, i) for i in range(len(KT))] + [(wubuf, i) for i in range(len(KT))]
        parts = []
        wo_prev = wobuf[(g + 3) % 4]
        for c in range(NCH):
            qproj(c)
            parts.append(up_piece(*pieces[len(parts)]))
            if c < len(pieces) - NCH:
                parts.append(up_piece(*pieces[len(parts)]))
            i = c - (NCH - NDEF)
            if i >= 0:
                acc_ref[:, pl.ds((NNOW + i) * TQ, TQ)] = deferred_oproj(i, wo_prev, g - 1)
        gate = sum(parts[1:len(KT)], parts[0])
        up = sum(parts[len(KT) + 1:], parts[len(KT)])
        hb_ref[...] = ((gate * jax.nn.sigmoid(gate)) * up).astype(_BF16)
        y = y_ref[...] * jax.nn.sigmoid(rsel_ref[:, 0:1])
        yt_ref[...] = jnp.concatenate(
            [y, jnp.zeros((128 - CP, D), _F32)], axis=0).T.astype(_BF16)

    for cp in cur[1:]:
        cp.wait()

    k = kbuf[slot]
    v = vbuf[slot]

    def qk(c, h):
        return jax.lax.dot_general(q_ref[c, :, h * DH:(h + 1) * DH], k, _NT,
                                   preferred_element_type=_F32)

    def pv(s):
        m = jnp.max(_tree(s, jnp.maximum), axis=-1, keepdims=True)
        p = jnp.exp2(s - m)
        tiles = [p[:, i * 128:(i + 1) * 128] for i in range(S // 128)]
        acc = None
        for g0 in range(0, len(tiles), 4):
            t = (tiles[g0] + tiles[g0 + 1]) + (tiles[g0 + 2] + tiles[g0 + 3])
            acc = t if acc is None else acc + t
            tiles[g0 + 3] = jnp.minimum(tiles[g0 + 3], acc)
        pb = jnp.concatenate(tiles, axis=-1).astype(_BF16)
        return jnp.dot(pb, v, preferred_element_type=_F32), acc

    hb = hb_ref[...]

    def down_piece(i):
        return jax.lax.dot_general(hb[:, i * 128:(i + 1) * 128],
                                   wdbuf[slot, :, i * 128:(i + 1) * 128], _NT,
                                   preferred_element_type=_F32)

    def prefetch():
        @pl.when(g + 1 < HKV)
        def _prefetch_attn():
            for cp in attn_copies(g + 1, 1 - slot):
                cp.start()

        @pl.when(g < NF)
        def _prefetch_moe():
            for cp in moe_copies(g, 1 - slot):
                cp.start()

    outs = []
    ys = []
    for c in range(NCH):
        sa = qk(c, 0)
        sb = qk(c, 1)
        ra, rb_ = pv(sa), pv(sb)
        if c == 0:
            prefetch()
        if c < FC // 128:
            ys.append(down_piece(c))
        if c < NNOW:
            outs.append((normalize(*ra), normalize(*rb_)))
        else:
            for h, r in enumerate((ra, rb_)):
                raw_ref[c - NNOW, h, 0] = r[0]
                raw_ref[c - NNOW, h, 1] = r[1]
    y_ref[...] += jnp.where(moe_active, sum(ys[1:], ys[0]), 0.0)
    wo_cur = wobuf[g % 4]
    for c in range(NNOW):
        acc_ref[:, pl.ds(c * TQ, TQ)] = oproj(c, *outs[c], wo_cur, g)

    @pl.when(g == HKV - 1)
    def _epilogue():
        yt = yt_ref[...]
        wo_last = wobuf[(HKV - 1) % 4]
        upds, late = [], []
        for c in range(NCH):
            if c >= NNOW:
                late.append(deferred_oproj(c - NNOW, wo_last, None))
            selc = jnp.concatenate(
                [sel_ref[:, pl.ds(c * TQ, TQ)], jnp.zeros((128 - CP, TQ), _BF16)], axis=0)
            upds.append(jnp.dot(yt, selc, preferred_element_type=_F32))
        for c in range(NCH):
            cols = pl.ds(c * TQ, TQ)
            attn = acc_ref[:, cols] if c < NNOW else late[c - NNOW]
            hb = 0.5 * (xnt_ref[:, cols].astype(_F32) + upds[c])
            gate = hb + hb * jnp.tanh(hb)
            obuf[:, cols] = (xt_ref[:, cols].astype(_F32) + attn * gate).astype(_BF16)
            out_copy(c).start()
        for c in range(NCH):
            out_copy(c).wait()


@jax.jit
def pallas_recurrent_scan__gqa_block_cached__moe_arch_mod__prompt_kernel(
    A_x: jax.Array,
    A_k_cache: jax.Array,
    A_v_cache: jax.Array,
    A_wq: jax.Array,
    A_wo: jax.Array,
    B_x: jax.Array,
    B_w_r: jax.Array,
    B_w_gate: jax.Array,
    B_w_up: jax.Array,
    B_w_down: jax.Array,
):
    xt = A_x.reshape(S, D).T
    k = A_k_cache.reshape(HKV, S, DH)
    v = A_v_cache.reshape(HKV, S, DH)
    wot = A_wo.T
    wdt = B_w_down.T

    out_t = pl.pallas_call(
        _kernel,
        grid=(HKV,),
        in_specs=[pl.BlockSpec(memory_space=pl.ANY)] * 9,
        out_specs=pl.BlockSpec(memory_space=pl.ANY),
        out_shape=jax.ShapeDtypeStruct((D, S), A_x.dtype),
        scratch_shapes=[
            pltpu.VMEM((D, S), _BF16),
            pltpu.VMEM((D,), _BF16),
            pltpu.VMEM((2, S, DH), _BF16),
            pltpu.VMEM((2, S, DH), _BF16),
            pltpu.VMEM((2, D, GW), _BF16),
            pltpu.VMEM((4, D, GW), _BF16),
            pltpu.VMEM((2, D, FC), _BF16),
            pltpu.VMEM((2, D, FC), _BF16),
            pltpu.VMEM((2, D, FC), _BF16),
            pltpu.VMEM((D, S), _BF16),
            pltpu.VMEM((S, D), _BF16),
            pltpu.VMEM((D, S), _BF16),
            pltpu.VMEM((D, S), _F32),
            pltpu.VMEM((CP, S), _BF16),
            pltpu.VMEM((CP, D), _BF16),
            pltpu.VMEM((CP, 128), _F32),
            pltpu.VMEM((CP, D), _F32),
            pltpu.VMEM((NDEF, REP, 2, TQ, 128), _F32),
            pltpu.VMEM((NCH, TQ, GW), _BF16),
            pltpu.VMEM((CP, FC), _BF16),
            pltpu.VMEM((D, 128), _BF16),
            pltpu.SemaphoreType.DMA((NCH,)),
            pltpu.SemaphoreType.DMA((NCH,)),
            pltpu.SemaphoreType.DMA((1,)),
            pltpu.SemaphoreType.DMA((2, 4)),
            pltpu.SemaphoreType.DMA((2, 3)),
        ],
        compiler_params=pltpu.CompilerParams(
            dimension_semantics=("arbitrary",),
            vmem_limit_bytes=126 * 1024 * 1024,
            disable_bounds_checks=True,
        ),
        name="fused_gqa_mod",
    )(xt, k, v, A_wq, wot, B_w_r, B_w_gate, B_w_up, wdt)
    return out_t.T.reshape(1, S, D)
```
